```python
import os as _os
_os.environ.setdefault('JAX_PLATFORMS', 'cpu')
import jax
import jax.numpy as jnp

def _softmax(x, axis=-1):
    return jax.nn.softmax(x, axis=axis)

def _gelu(x):
    return jax.nn.gelu(x, approximate=True)

def _silu(x):
    return jax.nn.silu(x)

def _sigmoid(x):
    return jax.nn.sigmoid(x)

def _layernorm(x, axis=-1, eps=1e-05):
    m = jnp.mean(x, axis=axis, keepdims=True)
    v = jnp.var(x, axis=axis, keepdims=True)
    return (x - m) / jnp.sqrt(v + eps)

def _scatter_add(tgt, idx, src, axis=0):
    return tgt.at[idx].add(src)

def _segment_sum(src, seg, n):
    return jax.ops.segment_sum(src, seg, n)

class _Rng:

    def __init__(self, key):
        self._k = key

    def _next(self):
        self._k, sub = jax.random.split(self._k)
        return sub

    def normal(self, shape):
        return jax.random.normal(self._next(), shape, dtype=jnp.bfloat16)

    def randint(self, lo, hi, shape):
        return jax.random.randint(self._next(), shape, lo, hi, dtype=jnp.int32)

    def uniform(self, shape, lo=0.0, hi=1.0):
        return jax.random.uniform(self._next(), shape, jnp.bfloat16, lo, hi)

    def permutation(self, n):
        return jax.random.permutation(self._next(), n)
kernel_name = 'adaLN_cond__sliding_block__dense_activation_relu__prompt'

def setup_inputs():
    _rng = _Rng(jax.random.key(int.from_bytes(__import__("os").urandom(4), "little")))
    _w = lambda a: (lambda t: t.astype(jnp.bfloat16) if jnp.issubdtype(t.dtype, jnp.floating) else t)(jnp.asarray(a))

    def _A_setup():
        B, S, D = (1, 2048, 512)
        return {'x': _w((lambda *s: _rng.normal(s) * 0.05)(B, S, D)), 'wqkv': _w((lambda *s: _rng.normal(s) * 0.05)(D, 3 * D)), 'wo': _w((lambda *s: _rng.normal(s) * 0.05)(D, D))}
    _A_in = _A_setup()

    def _B_setup():
        B, S, D, Dff = (1, 2048, 512, 1792)
        return {'x': _w((lambda *s: _rng.normal(s) * 0.05)(B, S, D)), 'w1': _w((lambda *s: _rng.normal(s) * 0.05)(D, Dff)), 'w2': _w((lambda *s: _rng.normal(s) * 0.05)(Dff, D))}
    _B_in = _B_setup()
    return {'A_x': _A_in['x'], 'A_wqkv': _A_in['wqkv'], 'A_wo': _A_in['wo'], 'B_x': _B_in['x'], 'B_w1': _B_in['w1'], 'B_w2': _B_in['w2'], 'c': _w((lambda *s: _rng.normal(s) * 0.05)(1, 512) * 8.0), 'w_mod': _w((lambda *s: _rng.normal(s) * 0.05)(512, 6 * 512) * 512 ** (-0.5) * 8.0)}

def reference(A_x, A_wqkv, A_wo, B_x, B_w1, B_w2, c, w_mod):

    def _A_ref(x, wqkv, wo):
        B, S, D = x.shape
        H = 32
        Dh = D // H
        W = 256
        qkv = (lambda x, *d: x.transpose(*d))((x @ wqkv).reshape(B, S, 3, H, Dh), 2, 0, 3, 1, 4)
        q, k, v = (qkv[0], qkv[1], qkv[2])
        scores = jnp.einsum('bhqd,bhkd->bhqk', q, k) * Dh ** (-0.5)
        idx = jnp.arange(S)
        mask = (idx[:, None] - idx[None, :] >= 0) & (idx[:, None] - idx[None, :] < W)
        scores = jnp.where(mask[None, None], scores, -1000000000.0)
        p = _softmax(scores, axis=-1)
        o = jnp.einsum('bhqk,bhkd->bhqd', p, v)
        return (lambda x, *d: x.transpose(*d))(o, 0, 2, 1, 3).reshape(B, S, D) @ wo

    def _B_ref(x, w1, w2):
        h = jnp.einsum('bsd,df->bsf', x, w1)
        zero = jnp.zeros_like(h)
        h = jnp.maximum(h, zero)
        return jnp.einsum('bsf,fd->bsd', h, w2)
    x = A_x
    mod = (_silu(c) @ w_mod).reshape(c.shape[0], 6, 1, -1)
    sa, ca, ga, sb, cb, gb = (mod[:, 0].copy(), mod[:, 1].copy(), mod[:, 2].copy(), mod[:, 3].copy(), mod[:, 4].copy(), mod[:, 5].copy())
    h = _layernorm(x, axis=-1) * (1 + ca) + sa
    x = x + ga * _A_ref(h, A_wqkv, A_wo)
    h = _layernorm(x, axis=-1) * (1 + cb) + sb
    x = x + gb * _B_ref(h, B_w1, B_w2)
    return x
```

```python
import jax
import jax.numpy as jnp
import jax.experimental.pallas as pl
import jax.experimental.pallas.tpu as pltpu

S = 2048
D = 512
H = 32
DH = 16
WIN = 256
DFF = 1792
EPS = 1e-5
NEG = -1e30
QSCALE = (DH ** -0.5) * 1.4426950408889634

TM = 256
NB = S // TM
QB = 128
NQ = S // QB
C = 8
B4 = 4
CPQ = H // C
NCH = NQ * CPQ

BF = jnp.bfloat16
F32 = jnp.float32
U32 = jnp.uint32

NT = (((1,), (1,)), ((), ()))
TN = (((0,), (0,)), ((), ()))


def _layernorm_mod(x, shift, scale1p):
    m = jnp.mean(x, axis=-1, keepdims=True)
    xc = x - m
    v = jnp.mean(xc * xc, axis=-1, keepdims=True)
    return xc * jax.lax.rsqrt(v + EPS) * scale1p + shift


def _kernel(x_hbm, wqkv_hbm, wo_hbm, w1_hbm, w2_hbm, c_hbm, wmod_hbm, o_hbm,
            x_v, wqkv_v, wqvt_v, wo_v, w1_v, w2_v, c_v, wmod_v, mod_v,
            ha, hb, k_s, qt_s, vt_s, ot_s, m2_s,
            sa, ma, sb, mb, pa, la, pb, lb,
            h2a, h2b, x1a, x1b, oa, ob, sems):
    def cp(src, dst, i):
        return pltpu.make_async_copy(src, dst, sems.at[i])

    d_c = cp(c_hbm, c_v, 0)
    d_wm0 = cp(wmod_hbm.at[:, pl.ds(0, 2 * D)], wmod_v.at[:, pl.ds(0, 2 * D)], 1)
    d_x0 = cp(x_hbm.at[0, pl.ds(0, TM), :], x_v.at[pl.ds(0, TM), :], 2)
    d_wk = cp(wqkv_hbm.at[:, pl.ds(D, D)], wqkv_v.at[:, pl.ds(D, D)], 3)
    d_wq = cp(wqkv_hbm.at[:, pl.ds(0, D)], wqkv_v.at[:, pl.ds(0, D)], 4)
    d_wv = cp(wqkv_hbm.at[:, pl.ds(2 * D, D)], wqkv_v.at[:, pl.ds(2 * D, D)], 5)
    d_x1 = cp(x_hbm.at[0, pl.ds(TM, S - TM), :], x_v.at[pl.ds(TM, S - TM), :], 6)
    d_wm1 = cp(wmod_hbm.at[:, pl.ds(2 * D, 4 * D)], wmod_v.at[:, pl.ds(2 * D, 4 * D)], 7)
    d_wo = cp(wo_hbm, wo_v, 8)
    d_w1 = cp(w1_hbm, w1_v, 9)
    d_w2 = cp(w2_hbm, w2_v, 10)
    for d in (d_c, d_wm0, d_x0, d_wq, d_wv, d_wk, d_x1):
        d.start()

    k_s[:, 0:WIN, :] = jnp.zeros((4, WIN, 128), BF)
    vt_s[0:2] = jnp.zeros((2, D, 128), BF)
    i2 = 2 * jax.lax.broadcasted_iota(jnp.int32, (64, 128), 0)
    al = jax.lax.broadcasted_iota(jnp.int32, (64, 128), 1)
    m2_s[...] = (jnp.where(i2 <= al, jnp.uint32(0xFFFF), jnp.uint32(0))
                 | jnp.where(i2 + 1 <= al, jnp.uint32(0xFFFF0000), jnp.uint32(0)))

    d_c.wait()
    cf = c_v[...].astype(F32)
    sc = (cf * (1.0 / (1.0 + jnp.exp(-cf)))).astype(BF)
    sc16 = jnp.broadcast_to(sc, (16, D))
    d_wm0.wait()
    mod_v[:, 0:2 * D] = jnp.dot(sc16, wmod_v[:, 0:2 * D], preferred_element_type=F32)[0:8]

    def ln1(b, h_ref):
        r0 = pl.multiple_of(b * TM, TM)
        x = x_v[pl.ds(r0, TM), :].astype(F32)
        h_ref[...] = _layernorm_mod(x, mod_v[0:1, 0:D], 1.0 + mod_v[0:1, D:2 * D]).astype(BF)

    d_x0.wait()
    ln1(0, ha)
    d_wq.wait()
    wqvt_v[0:D, :] = wqkv_v[:, 0:D].T
    d_wv.wait()
    wqvt_v[D:2 * D, :] = wqkv_v[:, 2 * D:3 * D].T
    d_wk.wait()
    d_x1.wait()
    for d in (d_wm1, d_wo, d_w1, d_w2):
        d.start()

    def proj(b, h_cur, h_nxt):
        h = h_cur[...]
        kk = jnp.dot(h, wqkv_v[:, D:2 * D], preferred_element_type=F32).astype(BF)
        r0 = pl.multiple_of(WIN + b * TM, TM)
        for g in range(4):
            k_s[g, pl.ds(r0, TM), :] = kk[:, g * 128:(g + 1) * 128]
        qv = jax.lax.dot_general(wqvt_v[...], h, NT, preferred_element_type=F32)
        for t in range(TM // QB):
            qt_s[b * (TM // QB) + t] = (qv[0:D, t * QB:(t + 1) * QB] * QSCALE).astype(BF)
            vt_s[2 + b * (TM // QB) + t] = qv[D:2 * D, t * QB:(t + 1) * QB].astype(BF)
        ln1(jnp.minimum(b + 1, NB - 1), h_nxt)

    def proj_body(b2, carry):
        proj(2 * b2, ha, hb)
        proj(2 * b2 + 1, hb, ha)
        return carry

    jax.lax.fori_loop(0, NB // 2, proj_body, 0)

    lane8 = jax.lax.broadcasted_iota(jnp.int32, (8, 128), 1)
    sub8 = jax.lax.broadcasted_iota(jnp.int32, (8, 128), 0)
    dd = lane8 - sub8
    k_u = k_s.bitcast(U32)
    qt_u = qt_s.bitcast(U32)
    vt_u = vt_s.bitcast(U32)

    def qk(c, s_ref, m_ref, j, masked):
        I = c // CPQ
        hbase = (c % CPQ) * C
        g = hbase // 8 + j // 8
        hh = j % 8
        h0 = pl.multiple_of(hbase * 8 + j * 8, 8)
        qt = pltpu.bitcast(qt_u[I, pl.ds(h0, 8), :], BF)
        parts = []
        if hh > 0:
            parts.append(jnp.zeros((16 * hh, 128), BF))
        parts.append(qt)
        if hh < 7:
            parts.append(jnp.zeros((16 * (7 - hh), 128), BF))
        wq = jnp.concatenate(parts, axis=0)
        kb = pl.multiple_of(I * 64, 64)
        pieces = []
        for r in range(8):
            pieces.append(k_u[g, pl.ds(kb + 8 * r, 8), :])
            pieces.append(k_u[g, pl.ds(kb + 128 + 8 * r, 8), :])
            pieces.append(k_u[g, pl.ds(kb + 64 + 8 * r, 8), :])
        kg = pltpu.bitcast(jnp.concatenate(pieces, axis=0), BF)
        st = jnp.dot(kg, wq, preferred_element_type=F32)
        mx = None
        for r in range(16):
            b = (r // 2) * 48 + (r % 2) * 8
            t0 = st[b: b + 8]
            t2 = st[b + 16: b + 24]
            t1 = st[b + 32: b + 40]
            if masked:
                t0 = jnp.where(I >= 2, t0, NEG)
                t1 = jnp.where(I >= 1, t1, NEG)
            mm = jnp.where(dd >= 8 * r, t2, t0)
            s_ref[j, 8 * r: 8 * r + 8, :] = mm
            s_ref[j, 128 + 8 * r: 128 + 8 * r + 8, :] = t1
            xm = jnp.maximum(mm, t1)
            mx = xm if mx is None else jnp.maximum(mx, xm)
        m = jnp.max(mx, axis=0, keepdims=True)
        m_ref[j] = jnp.broadcast_to(m, (8, 128))

    def sm(s_ref, m_ref, p_ref, l_ref, j):
        mrow = m_ref[j][0:1]
        pm = jnp.exp2(s_ref[j, 0:128, :] - mrow)
        p1 = jnp.exp2(s_ref[j, 128:256, :] - mrow)
        p_ref[j, 0:128, :] = pm.astype(BF)
        p_ref[j, 128:256, :] = p1.astype(BF)
        l = jnp.sum(pm + p1, axis=0, keepdims=True)
        l_ref[j] = jnp.broadcast_to(1.0 / l, (8, 128))

    def pv(c, p_ref, l_ref, j):
        I = c // CPQ
        hbase = (c % CPQ) * C
        h0 = pl.multiple_of(hbase * 8 + j * 8, 8)
        pu = p_ref.bitcast(U32)
        pm = pu[j, 0:64, :]
        p2 = pm & m2_s[...]
        p0 = pm ^ p2
        p = pltpu.bitcast(jnp.concatenate([p0, pu[j, 64:128, :], p2], axis=0), BF)
        vt = pltpu.bitcast(
            jnp.concatenate([vt_u[I + t, pl.ds(h0, 8), :] for t in range(3)], axis=1), BF)
        ot = jnp.dot(vt, p, preferred_element_type=F32)
        o0 = pl.multiple_of(hbase * 16 + j * 16, 16)
        ot_s[I, pl.ds(o0, 16), :] = (ot * l_ref[j][0:1]).astype(BF)

    def half(c, s_w, m_w, s_r, m_r, p_w, l_w, p_r, l_r, masked):
        c2 = jnp.minimum(c + 2, NCH - 1)
        for jj in range(0, C, B4):
            js = list(range(jj, jj + B4))
            for j in js:
                qk(c2, s_w, m_w, j, masked)
            for j in js:
                sm(s_r, m_r, p_w, l_w, j)
            for j in js:
                pv(c, p_r, l_r, j)

    def attn_body(masked):
        def body(c2, carry):
            c = 2 * c2
            half(c, sa, ma, sb, mb, pb, lb, pa, la, masked)
            half(c + 1, sb, mb, sa, ma, pa, la, pb, lb, masked)
            return carry
        return body

    for j in range(C):
        qk(0, sa, ma, j, True)
    for j in range(C):
        qk(1, sb, mb, j, True)
    for j in range(C):
        sm(sa, ma, pa, la, j)
    n_masked = CPQ - 1
    jax.lax.fori_loop(0, n_masked, attn_body(True), 0)
    jax.lax.fori_loop(n_masked, NCH // 2, attn_body(False), 0)

    d_wm1.wait()
    mod_v[:, 2 * D:6 * D] = jnp.dot(sc16, wmod_v[:, 2 * D:6 * D], preferred_element_type=F32)[0:8]
    d_wo.wait()
    d_w1.wait()
    d_w2.wait()
    ot_u = ot_s.bitcast(U32)

    def stage1(b, h2_ref, x1_ref):
        ot = pltpu.bitcast(
            jnp.concatenate([ot_u[b * (TM // QB) + t] for t in range(TM // QB)], axis=1), BF)
        att = jax.lax.dot_general(ot, wo_v[...], TN, preferred_element_type=F32)
        r0 = pl.multiple_of(b * TM, TM)
        x1 = x_v[pl.ds(r0, TM), :].astype(F32) + mod_v[0:1, 2 * D:3 * D] * att
        x1_ref[...] = x1
        h2_ref[...] = _layernorm_mod(x1, mod_v[0:1, 3 * D:4 * D], 1.0 + mod_v[0:1, 4 * D:5 * D]).astype(BF)

    def out_copy(b, o_ref, i):
        r0 = pl.multiple_of(b * TM, TM)
        return pltpu.make_async_copy(o_ref, o_hbm.at[0, pl.ds(r0, TM), :], sems.at[i])

    def stage2(b, h2_ref, x1_ref, o_ref):
        f = jnp.maximum(jnp.dot(h2_ref[...], w1_v[...], preferred_element_type=F32), 0.0).astype(BF)
        y = jnp.dot(f, w2_v[...], preferred_element_type=F32)
        o_ref[...] = (x1_ref[...] + mod_v[0:1, 5 * D:6 * D] * y).astype(BF)

    stage1(0, h2a, x1a)

    def ffn_pair(b, wait_prev):
        if wait_prev:
            out_copy(b - 2, oa, 11).wait()
        stage1(b + 1, h2b, x1b)
        stage2(b, h2a, x1a, oa)
        out_copy(b, oa, 11).start()
        if wait_prev:
            out_copy(b - 1, ob, 12).wait()
        stage1(jnp.minimum(b + 2, NB - 1), h2a, x1a)
        stage2(b + 1, h2b, x1b, ob)
        out_copy(b + 1, ob, 12).start()

    ffn_pair(0, False)

    def ffn_body(b2, carry):
        ffn_pair(2 * b2, True)
        return carry

    jax.lax.fori_loop(1, NB // 2, ffn_body, 0)
    out_copy(NB - 2, oa, 11).wait()
    out_copy(NB - 1, ob, 12).wait()


@jax.jit
def pallas_adaLN_cond__sliding_block__dense_activation_relu__prompt_kernel(
    A_x: jax.Array,
    A_wqkv: jax.Array,
    A_wo: jax.Array,
    B_x: jax.Array,
    B_w1: jax.Array,
    B_w2: jax.Array,
    c: jax.Array,
    w_mod: jax.Array,
):
    del B_x
    scratch = [
        pltpu.VMEM((S, D), BF),
        pltpu.VMEM((D, 3 * D), BF),
        pltpu.VMEM((2 * D, D), BF),
        pltpu.VMEM((D, D), BF),
        pltpu.VMEM((D, DFF), BF),
        pltpu.VMEM((DFF, D), BF),
        pltpu.VMEM((1, D), BF),
        pltpu.VMEM((D, 6 * D), BF),
        pltpu.VMEM((8, 6 * D), F32),
        pltpu.VMEM((TM, D), BF),
        pltpu.VMEM((TM, D), BF),
        pltpu.VMEM((4, S + WIN, 128), BF),
        pltpu.VMEM((NQ, D, 128), BF),
        pltpu.VMEM((NQ + 2, D, 128), BF),
        pltpu.VMEM((NQ, D, 128), BF),
        pltpu.VMEM((64, 128), U32),
        pltpu.VMEM((C, 256, 128), F32),
        pltpu.VMEM((C, 8, 128), F32),
        pltpu.VMEM((C, 256, 128), F32),
        pltpu.VMEM((C, 8, 128), F32),
        pltpu.VMEM((C, 256, 128), BF),
        pltpu.VMEM((C, 8, 128), F32),
        pltpu.VMEM((C, 256, 128), BF),
        pltpu.VMEM((C, 8, 128), F32),
        pltpu.VMEM((TM, D), BF),
        pltpu.VMEM((TM, D), BF),
        pltpu.VMEM((TM, D), F32),
        pltpu.VMEM((TM, D), F32),
        pltpu.VMEM((TM, D), BF),
        pltpu.VMEM((TM, D), BF),
        pltpu.SemaphoreType.DMA((13,)),
    ]
    return pl.pallas_call(
        _kernel,
        out_shape=jax.ShapeDtypeStruct((1, S, D), BF),
        in_specs=[pl.BlockSpec(memory_space=pl.ANY)] * 7,
        out_specs=pl.BlockSpec(memory_space=pl.ANY),
        scratch_shapes=scratch,
        compiler_params=pltpu.CompilerParams(vmem_limit_bytes=100 * 1024 * 1024),
        name="adaln_swa_ffn",
    )(A_x, A_wqkv, A_wo, B_w1, B_w2, c, w_mod)
```

```python
import jax
import jax.numpy as jnp
import jax.experimental.pallas as pl
import jax.experimental.pallas.tpu as pltpu

S = 2048
D = 512
H = 32
DH = 16
WIN = 256
DFF = 1792
EPS = 1e-5
NEG = -1e30
QSCALE = (DH ** -0.5) * 1.4426950408889634

TM = 256
NB = S // TM
QB = 128
NQ = S // QB
C = 16
B4 = 4
CPQ = H // C
NCH = NQ * CPQ

SCHED = {0: [0], 1: [1], 2: [2], 3: [3], 4: [4]}

BF = jnp.bfloat16
F32 = jnp.float32
U32 = jnp.uint32

NT = (((1,), (1,)), ((), ()))
TN = (((0,), (0,)), ((), ()))
TT = (((0,), (1,)), ((), ()))


def _ldp(ref, p0, p1, r0=None, r1=None):
    u = ref.bitcast(U32)
    if r0 is None:
        r0, r1 = 0, ref.shape[1]
    return pltpu.bitcast(
        jnp.concatenate([u[p, r0 // 2:r1 // 2, :] for p in range(p0, p1)], axis=1), BF)


def _mult(x, m):
    return x if isinstance(x, int) else pl.multiple_of(x, m)


def _normalize(x):
    m = jnp.mean(x, axis=-1, keepdims=True)
    xc = x - m
    v = jnp.mean(xc * xc, axis=-1, keepdims=True)
    return xc * jax.lax.rsqrt(v + EPS)


def _layernorm_mod(x, shift, scale1p):
    return _normalize(x) * scale1p + shift


def _kernel(x_hbm, wqkv_hbm, wo_hbm, w1_hbm, w2_hbm, c_hbm, wmod_hbm, o_hbm,
            x_v, wqkv_v, wo_v, w1_v, w2_v, c_v, wmod_v, mod_v,
            ha, hb, k_s, qt_s, vt_s, ot_s, m2_s,
            sa, ma, sb, mb, pa, la, pb, lb,
            o_v, on_s, sems, osems):
    def cp(src, dst, i):
        return pltpu.make_async_copy(src, dst, sems.at[i])

    d_c = cp(c_hbm, c_v, 0)
    d_wm0 = cp(wmod_hbm.at[:, pl.ds(0, 2 * D)], wmod_v.at[:, pl.ds(0, 2 * D)], 1)
    d_x0 = cp(x_hbm.at[0, pl.ds(0, TM), :], x_v.at[pl.ds(0, TM), :], 2)
    def panels(src, dst, n0, n1, sem0, off=0):
        return [cp(src.at[:, pl.ds(n * 128, 128)], dst.at[n - off], sem0 + n - n0) for n in range(n0, n1)]

    d_wq = panels(wqkv_hbm, wqkv_v, 0, 4, 16)
    d_wk = panels(wqkv_hbm, wqkv_v, 4, 8, 20)
    d_wv = panels(wqkv_hbm, wqkv_v, 8, 12, 24)
    d_x1 = cp(x_hbm.at[0, pl.ds(TM, TM), :], x_v.at[pl.ds(TM, TM), :], 6)
    d_x2 = cp(x_hbm.at[0, pl.ds(2 * TM, TM), :], x_v.at[pl.ds(2 * TM, TM), :], 3)
    d_x3 = cp(x_hbm.at[0, pl.ds(3 * TM, S - 3 * TM), :], x_v.at[pl.ds(3 * TM, S - 3 * TM), :], 4)
    d_wm1 = cp(wmod_hbm.at[:, pl.ds(2 * D, 4 * D)], wmod_v.at[:, pl.ds(2 * D, 4 * D)], 7)
    d_wo = panels(wo_hbm, wo_v, 0, 4, 28)
    d_w1 = panels(w1_hbm, w1_v, 0, 14, 32)
    d_w2 = panels(w2_hbm, w2_v, 0, 4, 46)
    for d in [d_c, d_x0, d_wm0] + d_wk + [d_x1] + d_wq + d_wv + [d_x2, d_x3]:
        d.start()

    k_s[:, 0:WIN, :] = jnp.zeros((4, WIN, 128), BF)
    vt_s[0:2] = jnp.zeros((2, D, 128), BF)
    pa[:, 128:256, :] = jnp.zeros((C, 128, 128), BF)
    pb[:, 128:256, :] = jnp.zeros((C, 128, 128), BF)
    i2 = 2 * jax.lax.broadcasted_iota(jnp.int32, (64, 128), 0)
    al = jax.lax.broadcasted_iota(jnp.int32, (64, 128), 1)
    m2_s[...] = (jnp.where(i2 <= al, jnp.uint32(0xFFFF), jnp.uint32(0))
                 | jnp.where(i2 + 1 <= al, jnp.uint32(0xFFFF0000), jnp.uint32(0)))

    d_c.wait()
    d_x0.wait()
    cf = c_v[...].astype(F32)
    sc = (cf * (1.0 / (1.0 + jnp.exp(-cf)))).astype(BF)
    sc16 = jnp.broadcast_to(sc, (16, D))
    n0 = _normalize(x_v[0:TM, :].astype(F32))
    d_wm0.wait()
    mod_v[:, 0:2 * D] = jnp.dot(sc16, wmod_v[:, 0:2 * D], preferred_element_type=F32)[0:8]

    def put_h(n, h_ref):
        h = (n * (1.0 + mod_v[0:1, D:2 * D]) + mod_v[0:1, 0:D]).astype(BF)
        for p in range(4):
            h_ref[p] = h[:, p * 128:(p + 1) * 128]

    def ln1(b, h_ref):
        r0 = pl.multiple_of(b * TM, TM)
        put_h(_normalize(x_v[pl.ds(r0, TM), :].astype(F32)), h_ref)

    def proj_k(b, h_cur):
        h = _ldp(h_cur, 0, 4)
        kk = jnp.dot(h, _ldp(wqkv_v, 4, 8), preferred_element_type=F32).astype(BF)
        r0 = pl.multiple_of(WIN + b * TM, TM)
        for g in range(4):
            k_s[g, pl.ds(r0, TM), :] = kk[:, g * 128:(g + 1) * 128]

    def proj_qv(b, h_cur):
        h = _ldp(h_cur, 0, 4)
        wqv = jnp.concatenate([_ldp(wqkv_v, 0, 4), _ldp(wqkv_v, 8, 12)], axis=1)
        qv = jax.lax.dot_general(wqv, h, TT, preferred_element_type=F32)
        for t in range(TM // QB):
            qt_s[b * (TM // QB) + t] = (qv[0:D, t * QB:(t + 1) * QB] * QSCALE).astype(BF)
            vt_s[2 + b * (TM // QB) + t] = qv[D:2 * D, t * QB:(t + 1) * QB].astype(BF)

    def proj(b, h_cur, h_nxt):
        ln1(jnp.minimum(b + 1, NB - 1), h_nxt)
        proj_k(b, h_cur)
        proj_qv(b, h_cur)

    put_h(n0, ha)
    for d in d_wk + [d_x1]:
        d.wait()
    proj_k(0, ha)
    ln1(1, hb)
    proj_k(1, hb)
    for d in d_wq + d_wv + [d_x2]:
        d.wait()
    for d in [d_wm1] + d_wo + d_w1 + d_w2:
        d.start()
    proj_qv(0, ha)
    ln1(2, ha)
    proj_qv(1, hb)
    d_x3.wait()

    def proj_body(b2, carry):
        proj(2 * b2, ha, hb)
        proj(2 * b2 + 1, hb, ha)
        return carry

    jax.lax.fori_loop(1, NB // 2, proj_body, 0)

    lane8 = jax.lax.broadcasted_iota(jnp.int32, (8, 128), 1)
    sub8 = jax.lax.broadcasted_iota(jnp.int32, (8, 128), 0)
    dd = lane8 - sub8
    k_u = k_s.bitcast(U32)
    qt_u = qt_s.bitcast(U32)
    vt_u = vt_s.bitcast(U32)

    def qk(c, s_ref, m_ref, j, nblk=3):
        I = c // CPQ
        hbase = (c % CPQ) * C
        g = hbase // 8 + j // 8
        hh = j % 8
        h0 = _mult(hbase * 8 + j * 8, 8)
        qt = pltpu.bitcast(qt_u[I, pl.ds(h0, 8), :], BF)
        parts = []
        if hh > 0:
            parts.append(jnp.zeros((16 * hh, 128), BF))
        parts.append(qt)
        if hh < 7:
            parts.append(jnp.zeros((16 * (7 - hh), 128), BF))
        wq = jnp.concatenate(parts, axis=0)
        kb = _mult(I * 64, 64)
        offs = {3: (128, 0, 64), 2: (128, 64), 1: (128,)}[nblk]
        if nblk == 3:
            offs = (0, 128, 64)
        pieces = []
        for r in range(8):
            for o in offs:
                pieces.append(k_u[g, pl.ds(kb + o + 8 * r, 8), :])
        kg = pltpu.bitcast(jnp.concatenate(pieces, axis=0), BF)
        st = jnp.dot(kg, wq, preferred_element_type=F32)
        mx = None
        for r in range(16):
            b = (r // 2) * 16 * nblk + (r % 2) * 8
            blk = {o: st[b + 16 * i: b + 16 * i + 8] for i, o in enumerate(offs)}
            mm = jnp.where(dd >= 8 * r, blk[128], blk[0] if nblk == 3 else NEG)
            s_ref[j, 8 * r: 8 * r + 8, :] = mm
            xm = mm
            if nblk >= 2:
                s_ref[j, 128 + 8 * r: 128 + 8 * r + 8, :] = blk[64]
                xm = jnp.maximum(mm, blk[64])
            mx = xm if mx is None else jnp.maximum(mx, xm)
        m = jnp.max(mx, axis=0, keepdims=True)
        m_ref[j] = jnp.broadcast_to(m, (8, 128))

    def sm(s_ref, m_ref, p_ref, l_ref, j, first=False):
        mrow = m_ref[j][0:1]
        pm = jnp.exp2(s_ref[j, 0:128, :] - mrow)
        p_ref[j, 0:128, :] = pm.astype(BF)
        if not first:
            p1 = jnp.exp2(s_ref[j, 128:256, :] - mrow)
            p_ref[j, 128:256, :] = p1.astype(BF)
            pm = pm + p1
        l = jnp.sum(pm, axis=0, keepdims=True)
        l_ref[j] = jnp.broadcast_to(1.0 / l, (8, 128))

    def pv_first(c, p_ref, l_ref, j):
        h0 = (c % CPQ) * C * 8 + j * 8
        p = pltpu.bitcast(p_ref.bitcast(U32)[j, 0:64, :], BF)
        vt = pltpu.bitcast(vt_u[2, pl.ds(h0, 8), :], BF)
        ot = jnp.dot(vt, p, preferred_element_type=F32)
        ot_s[0, pl.ds(2 * h0, 16), :] = (ot * l_ref[j][0:1]).astype(BF)

    def pv_tile(c, p_ref, l_ref, j, t, acc):
        I = c // CPQ
        hbase = (c % CPQ) * C
        h0 = _mult(hbase * 8 + j * 8, 8)
        pu = p_ref.bitcast(U32)
        if t == 1:
            p = pu[j, 64:128, :]
        else:
            pm = pu[j, 0:64, :]
            p2 = pm & m2_s[...]
            p = p2 if t == 2 else pm ^ p2
        vt = pltpu.bitcast(vt_u[I + t, pl.ds(h0, 8), :], BF)
        ot = jnp.dot(vt, pltpu.bitcast(p, BF), preferred_element_type=F32)
        acc = ot if acc is None else acc + ot
        if t == 2:
            o0 = _mult(hbase * 16 + j * 16, 16)
            ot_s[I, pl.ds(o0, 16), :] = (acc * l_ref[j][0:1]).astype(BF)
        return acc

    ot_u = ot_s.bitcast(U32)

    def dense_pieces(b):
        st = {}
        r0 = _mult(b * QB, QB)
        ot = pltpu.bitcast(ot_u[b], BF)
        for n in range(4):
            on_s[n] = ot[n * 128:(n + 1) * 128, :].T

        def p_wo(n):
            def run():
                att = jnp.dot(_ldp(on_s, 0, 4), _ldp(wo_v, n, n + 1), preferred_element_type=F32)
                st.setdefault("att", []).append(att)
                if n == 3:
                    att = jnp.concatenate(st["att"], axis=1)
                    x1 = x_v[pl.ds(r0, QB), :].astype(F32) + mod_v[0:1, 2 * D:3 * D] * att
                    st["x1"] = x1
                    st["h2"] = _layernorm_mod(
                        x1, mod_v[0:1, 3 * D:4 * D], 1.0 + mod_v[0:1, 4 * D:5 * D]).astype(BF)
            return run

        def p_w1(n):
            def run():
                f = jnp.dot(st["h2"], _ldp(w1_v, n, n + 1), preferred_element_type=F32)
                st.setdefault("f", []).append(jnp.maximum(f, 0.0).astype(BF))
            return run

        def p_w2(c, n0, n1):
            k0, k1 = 4 * c, min(4 * c + 4, 14)

            def run():
                f = jnp.concatenate(st["f"][k0:k1], axis=1)
                y = jnp.dot(f, _ldp(w2_v, n0, n1, k0 * 128, k1 * 128), preferred_element_type=F32)
                for n in range(n0, n1):
                    yn = y[:, (n - n0) * 128:(n - n0 + 1) * 128]
                    if c > 0:
                        yn = st["y", n] + yn
                    st["y", n] = yn
                    if c == 3:
                        cs = slice(n * 128, (n + 1) * 128)
                        o_v[pl.ds(r0, QB), cs] = (
                            st["x1"][:, cs] + mod_v[0:1, 5 * D + n * 128:5 * D + (n + 1) * 128] * yn
                        ).astype(BF)
            return run

        w1 = [p_w1(n) for n in range(14)]
        w2 = {(c, n): p_w2(c, n, n + 1) for c in range(3) for n in range(4)}
        seq = [p_wo(n) for n in range(4)] + w1[0:4]
        for i in range(8):
            seq += [w1[4 + i], w2[(i // 4, i % 4)]]
        seq += [w1[12], w1[13], w2[(2, 0)], w2[(2, 1)], w2[(2, 2)], w2[(2, 3)],
                p_w2(3, 0, 2), p_w2(3, 2, 4)]
        return seq

    def out_copy(b):
        r0 = _mult(b * QB, QB)
        return pltpu.make_async_copy(o_v.at[pl.ds(r0, QB), :], o_hbm.at[0, pl.ds(r0, QB), :], osems.at[b])

    def pv_group(c, js, p_r, l_r, between):
        acc = {j: None for j in js}
        for t in range(4):
            between[t]()
            if t < 3:
                for j in js:
                    acc[j] = pv_tile(c, p_r, l_r, j, t, acc[j])

    bufs = ((sa, ma, pa, la), (sb, mb, pb, lb))

    def step(I):
        pieces = dense_pieces(I - 1)
        for k in range(8):
            half, js = k // 4, list(range((k % 4) * B4, (k % 4 + 1) * B4))
            c = 2 * I + half
            s_w, m_w, p_r, l_r = bufs[half]
            s_r, m_r, p_w, l_w = bufs[1 - half]
            for j in js:
                qk(c + 2, s_w, m_w, j)

            def slot(t, k=k, js=js, s_r=s_r, m_r=m_r, p_w=p_w, l_w=l_w):
                def run():
                    if t > 0:
                        sm(s_r, m_r, p_w, l_w, js[t - 1])
                    pieces[4 * k + t]()
                return run

            pv_group(c, js, p_r, l_r, [slot(t) for t in range(4)])
            sm(s_r, m_r, p_w, l_w, js[3])
        out_copy(I - 1).start()

    for d in [d_wm1] + d_wo + d_w1 + d_w2:
        d.wait()

    def mod2(n):
        cs = slice(2 * D + n * 128, 2 * D + (n + 1) * 128)
        mod_v[:, cs] = jnp.dot(sc16, wmod_v[:, cs], preferred_element_type=F32)[0:8]

    grp = [list(range(g * B4, (g + 1) * B4)) for g in range(4)]
    for js in grp:
        for j in js:
            qk(0, sa, ma, j, 1)
    for js in grp:
        for j in js:
            qk(1, sb, mb, j, 1)
        for j in js:
            sm(sa, ma, pa, la, j, first=True)
    for g, js in enumerate(grp):
        for j in js:
            qk(2, sa, ma, j, 2)
        mod2(2 * g)
        for j in js:
            pv_first(0, pa, la, j)
        mod2(2 * g + 1)
        for j in js:
            sm(sb, mb, pb, lb, j, first=True)
    for g, js in enumerate(grp):
        for j in js:
            qk(3, sb, mb, j, 2)
        mod2(8 + 2 * g)
        for j in js:
            pv_first(1, pb, lb, j)
        mod2(9 + 2 * g)
        for j in js:
            sm(sa, ma, pa, la, j)

    def body(I, carry):
        step(I)
        return carry

    jax.lax.fori_loop(1, NQ - 1, body, 0)
    def nop():
        pass

    b14 = dense_pieces(NQ - 2)
    for p in b14[0:4]:
        p()
    for js in grp:
        pv_group(NCH - 2, js, pa, la,
                 [nop] + [lambda j=j: sm(sb, mb, pb, lb, j) for j in js[0:3]])
        sm(sb, mb, pb, lb, js[3])
    for js in grp:
        pv_group(NCH - 1, js, pb, lb, [nop] * 4)
    for p in b14[4:8]:
        p()
    b15 = dense_pieces(NQ - 1)
    for p in b15[0:4]:
        p()
    for p in b14[8:32]:
        p()
    for p in b15[4:8]:
        p()
    out_copy(NQ - 2).start()
    for p in b15[8:32]:
        p()
    out_copy(NQ - 1).start()
    for b in range(NQ):
        out_copy(b).wait()


@jax.jit
def pallas_adaLN_cond__sliding_block__dense_activation_relu__prompt_kernel(
    A_x: jax.Array,
    A_wqkv: jax.Array,
    A_wo: jax.Array,
    B_x: jax.Array,
    B_w1: jax.Array,
    B_w2: jax.Array,
    c: jax.Array,
    w_mod: jax.Array,
):
    del B_x
    scratch = [
        pltpu.VMEM((S, D), BF),
        pltpu.VMEM((12, D, 128), BF),
        pltpu.VMEM((4, D, 128), BF),
        pltpu.VMEM((14, D, 128), BF),
        pltpu.VMEM((4, DFF, 128), BF),
        pltpu.VMEM((1, D), BF),
        pltpu.VMEM((D, 6 * D), BF),
        pltpu.VMEM((8, 6 * D), F32),
        pltpu.VMEM((4, TM, 128), BF),
        pltpu.VMEM((4, TM, 128), BF),
        pltpu.VMEM((4, S + WIN, 128), BF),
        pltpu.VMEM((NQ, D, 128), BF),
        pltpu.VMEM((NQ + 2, D, 128), BF),
        pltpu.VMEM((NQ, D, 128), BF),
        pltpu.VMEM((64, 128), U32),
        pltpu.VMEM((C, 256, 128), F32),
        pltpu.VMEM((C, 8, 128), F32),
        pltpu.VMEM((C, 256, 128), F32),
        pltpu.VMEM((C, 8, 128), F32),
        pltpu.VMEM((C, 256, 128), BF),
        pltpu.VMEM((C, 8, 128), F32),
        pltpu.VMEM((C, 256, 128), BF),
        pltpu.VMEM((C, 8, 128), F32),
        pltpu.VMEM((S, D), BF),
        pltpu.VMEM((4, QB, 128), BF),
        pltpu.SemaphoreType.DMA((50,)),
        pltpu.SemaphoreType.DMA((NQ,)),
    ]
    return pl.pallas_call(
        _kernel,
        out_shape=jax.ShapeDtypeStruct((1, S, D), BF),
        in_specs=[pl.BlockSpec(memory_space=pl.ANY)] * 7,
        out_specs=pl.BlockSpec(memory_space=pl.ANY),
        scratch_shapes=scratch,
        compiler_params=pltpu.CompilerParams(vmem_limit_bytes=100 * 1024 * 1024),
        name="adaln_swa_ffn",
    )(A_x, A_wqkv, A_wo, B_w1, B_w2, c, w_mod)
```

```python
import jax
import jax.numpy as jnp
import jax.experimental.pallas as pl
import jax.experimental.pallas.tpu as pltpu

S = 2048
D = 512
H = 32
DH = 16
WIN = 256
DFF = 1792
EPS = 1e-5
NEG = -1e30
QSCALE = (DH ** -0.5) * 1.4426950408889634

TM = 256
NB = S // TM
QB = 128
NQ = S // QB
NP = H // 2
NG = 8
NBUF = 2
LS = 1
WOPOS = 8
LQ = 2

BF = jnp.bfloat16
F32 = jnp.float32
U32 = jnp.uint32

TT = (((0,), (1,)), ((), ()))


def _ldp(ref, p0, p1, r0=None, r1=None):
    u = ref.bitcast(U32)
    if r0 is None:
        r0, r1 = 0, ref.shape[1]
    return pltpu.bitcast(
        jnp.concatenate([u[p, r0 // 2:r1 // 2, :] for p in range(p0, p1)], axis=1), BF)


def _mult(x, m):
    return x if isinstance(x, int) else pl.multiple_of(x, m)


class _Blk:
    def __init__(self, value, parity):
        self.value, self.parity = value, parity

    def __mul__(self, k):
        return self.value * k


def _normalize(x):
    m = jnp.mean(x, axis=-1, keepdims=True)
    xc = x - m
    v = jnp.mean(xc * xc, axis=-1, keepdims=True)
    return xc * jax.lax.rsqrt(v + EPS)


def _layernorm_mod(x, shift, scale1p):
    return _normalize(x) * scale1p + shift


def _kernel(x_hbm, wqkv_hbm, wo_hbm, w1_hbm, w2_hbm, c_hbm, wmod_hbm, o_hbm,
            x_v, wqkv_v, wo_v, w1_v, w2_v, c_v, wmod_v, mod_v,
            ha, hb, k_s, qt_s, vt_s, ot_s, m2_s,
            o_v, on_s, x1a, h2a, x1b, h2b, sems, osems, *bufs):
    def cp(src, dst, i):
        return pltpu.make_async_copy(src, dst, sems.at[i])

    d_c = cp(c_hbm, c_v, 0)
    d_wm0 = cp(wmod_hbm.at[:, pl.ds(0, 2 * D)], wmod_v.at[:, pl.ds(0, 2 * D)], 1)
    d_x0 = cp(x_hbm.at[0, pl.ds(0, TM), :], x_v.at[pl.ds(0, TM), :], 2)
    def panels(src, dst, n0, n1, sem0, off=0):
        return [cp(src.at[:, pl.ds(n * 128, 128)], dst.at[n - off], sem0 + n - n0) for n in range(n0, n1)]

    d_wq = panels(wqkv_hbm, wqkv_v, 0, 4, 16)
    d_wk = panels(wqkv_hbm, wqkv_v, 4, 8, 20)
    d_wv = panels(wqkv_hbm, wqkv_v, 8, 12, 24)
    d_x1 = cp(x_hbm.at[0, pl.ds(TM, TM), :], x_v.at[pl.ds(TM, TM), :], 6)
    d_x2 = cp(x_hbm.at[0, pl.ds(2 * TM, TM), :], x_v.at[pl.ds(2 * TM, TM), :], 3)
    d_x3 = cp(x_hbm.at[0, pl.ds(3 * TM, S - 3 * TM), :], x_v.at[pl.ds(3 * TM, S - 3 * TM), :], 4)
    d_wm1 = cp(wmod_hbm.at[:, pl.ds(2 * D, 4 * D)], wmod_v.at[:, pl.ds(2 * D, 4 * D)], 7)
    d_wo = panels(wo_hbm, wo_v, 0, 4, 28)
    d_w1 = panels(w1_hbm, w1_v, 0, 14, 32)
    d_w2 = panels(w2_hbm, w2_v, 0, 4, 46)
    for d in [d_c, d_x0, d_wm0] + d_wk + [d_x1] + d_wq + d_wv + [d_x2, d_x3]:
        d.start()

    bufs = [bufs[8 * b:8 * b + 8] for b in range(NBUF)]
    s_bufs = [((se, me), (so, mo)) for se, me, so, mo, _, _, _, _ in bufs]
    p_bufs = [b[4:6] for b in bufs]
    l_bufs = [b[6:8] for b in bufs]
    for b in p_bufs:
        for p_ref in b:
            p_ref[...] = jnp.zeros((2, 256, 128), BF)
    i2 = 2 * jax.lax.broadcasted_iota(jnp.int32, (32, 128), 0)
    al = jax.lax.broadcasted_iota(jnp.int32, (32, 128), 1) & 63
    m2_s[...] = (jnp.where(i2 <= al, jnp.uint32(0xFFFF), jnp.uint32(0))
                 | jnp.where(i2 + 1 <= al, jnp.uint32(0xFFFF0000), jnp.uint32(0)))

    d_c.wait()
    d_x0.wait()
    cf = c_v[...].astype(F32)
    sc = (cf * (1.0 / (1.0 + jnp.exp(-cf)))).astype(BF)
    sc16 = jnp.broadcast_to(sc, (16, D))
    n0 = _normalize(x_v[0:TM, :].astype(F32))
    d_wm0.wait()
    mod_v[:, 0:2 * D] = jnp.dot(sc16, wmod_v[:, 0:2 * D], preferred_element_type=F32)[0:8]

    def put_h(n, h_ref):
        h = (n * (1.0 + mod_v[0:1, D:2 * D]) + mod_v[0:1, 0:D]).astype(BF)
        for p in range(4):
            h_ref[p] = h[:, p * 128:(p + 1) * 128]

    def ln1(b, h_ref):
        r0 = pl.multiple_of(b * TM, TM)
        put_h(_normalize(x_v[pl.ds(r0, TM), :].astype(F32)), h_ref)

    def proj_k(b, h_cur):
        h = _ldp(h_cur, 0, 4)
        kk = jnp.dot(h, _ldp(wqkv_v, 4, 8), preferred_element_type=F32).astype(BF)
        r0 = _mult(b * TM, TM)
        for g in range(4):
            k_s[g, pl.ds(r0, TM), :] = kk[:, g * 128:(g + 1) * 128]

    def proj_qv(b, h_cur):
        h = _ldp(h_cur, 0, 4)
        wqv = jnp.concatenate([_ldp(wqkv_v, 0, 4), _ldp(wqkv_v, 8, 12)], axis=1)
        qv = jax.lax.dot_general(wqv, h, TT, preferred_element_type=F32)
        for t in range(TM // QB):
            q = qv[0:D, t * QB:(t + 1) * QB] * QSCALE
            q = jnp.concatenate(
                [q[16 * h:16 * h + 16] if h % 2 == 0 else pltpu.roll(q[16 * h:16 * h + 16], 64, 1)
                 for h in range(H)], axis=0)
            qt_s[b * (TM // QB) + t] = q.astype(BF)
            vt_s[b * (TM // QB) + t] = qv[D:2 * D, t * QB:(t + 1) * QB].astype(BF)

    def proj(b, h_cur, h_nxt):
        ln1(jnp.minimum(b + 1, NB - 1), h_nxt)
        proj_k(b, h_cur)
        proj_qv(b, h_cur)

    put_h(n0, ha)
    for d in d_wk + [d_x1]:
        d.wait()
    proj_k(0, ha)
    ln1(1, hb)
    proj_k(1, hb)
    for d in d_wq + d_wv + [d_x2]:
        d.wait()
    for d in [d_wm1] + d_wo + d_w1 + d_w2:
        d.start()
    proj_qv(0, ha)
    ln1(2, ha)
    proj_qv(1, hb)
    d_x3.wait()

    def proj_body(b2, carry):
        proj(2 * b2, ha, hb)
        proj(2 * b2 + 1, hb, ha)
        return carry

    jax.lax.fori_loop(1, NB // 2, proj_body, 0)

    lane8 = jax.lax.broadcasted_iota(jnp.int32, (8, 128), 1)
    sub8 = jax.lax.broadcasted_iota(jnp.int32, (8, 128), 0)
    dd = (lane8 & 63) - sub8
    lo8 = lane8 < 64
    lo32 = jax.lax.broadcasted_iota(jnp.int32, (32, 128), 1) < 64
    lo1 = jax.lax.broadcasted_iota(jnp.int32, (1, 128), 1) < 64

    k_u = k_s.bitcast(U32)
    qt_u = qt_s.bitcast(U32)
    vt_u = vt_s.bitcast(U32)
    ot_u = ot_s.bitcast(U32)
    pu_bufs = [[r.bitcast(U32) for r in rs] for rs in p_bufs]

    def first_valid(I, e):
        return max(0, WIN - 64 * (2 * I + e)) if isinstance(I, int) else 0

    def qk(I, e, p):
        s_ref, m_ref = s_bufs[p // 2 % NBUF][e]
        j = p % 2
        g, q = p // 4, p % 4
        qa = qt_u[I, 16 * p:16 * p + 8, :]
        qb = qt_u[I, 16 * p + 8:16 * p + 16, :]
        zero = jnp.zeros((8, 128), U32)
        if e == 0:
            qa, qb = jnp.where(lo8, qa, zero), jnp.where(lo8, zero, qb)
        else:
            qa, qb = jnp.where(lo8, zero, qa), jnp.where(lo8, qb, zero)
        parts = [zero] * (2 * q) + [qa, qb] + [zero] * (6 - 2 * q)
        wq = pltpu.bitcast(jnp.concatenate(parts, axis=0), BF)
        lo = first_valid(I, e)
        rows = []
        for r in range(4):
            rows += [16 * r, WIN + 16 * r] + [64 + 16 * (3 * r + i) for i in range(3)]
        rows = [o for o in rows if o >= lo]
        kb = (2 * I + e) * 32 - WIN // 2
        kg = pltpu.bitcast(jnp.concatenate(
            [k_u[g, pl.ds(_mult(kb + o // 2, 8), 8), :] for o in rows], axis=0), BF)
        st = jnp.dot(kg, wq, preferred_element_type=F32)
        blk = {o + 8 * h: st[16 * i + 8 * h:16 * i + 8 * h + 8] for i, o in enumerate(rows) for h in range(2)}
        mx = [None, None]
        for i, o in enumerate(rows):
            for h in range(2):
                mu = o + 8 * h
                if mu < 64:
                    continue
                if mu >= WIN:
                    mu -= WIN
                    v = jnp.where(dd >= mu, blk[WIN + mu], blk[mu] if mu in blk else NEG)
                else:
                    v = blk[mu]
                s_ref[j, mu:mu + 8, :] = v
                mx[h] = v if mx[h] is None else jnp.maximum(mx[h], v)
        m = jnp.max(jnp.maximum(mx[0], mx[1]), axis=0, keepdims=True)
        m_ref[j] = jnp.broadcast_to(m, (8, 128))

    def sm(I, p):
        li = []
        b, j = p // 2 % NBUF, p % 2
        for e in range(2):
            (s_ref, m_ref), p_ref = s_bufs[b][e], p_bufs[b][e]
            mrow = m_ref[j][0:1]
            lvl = []
            for r in range(16):
                if r < 4 or 16 * r >= first_valid(I, e):
                    pj = jnp.exp2(s_ref[j, 16 * r:16 * r + 16, :] - mrow)
                    p_ref[j, 16 * r:16 * r + 16, :] = pj.astype(BF)
                    lvl.append(pj[0:8] + pj[8:16])
            while len(lvl) > 1:
                lvl = [lvl[i] + lvl[i + 1] if i + 1 < len(lvl) else lvl[i] for i in range(0, len(lvl), 2)]
            tot = lvl[0]
            li.append(1.0 / jnp.sum(tot, axis=0, keepdims=True))
        l_bufs[b][0][j] = jnp.broadcast_to(jnp.where(lo1, li[0], li[1]), (8, 128))
        l_bufs[b][1][j] = jnp.broadcast_to(jnp.where(lo1, li[1], li[0]), (8, 128))

    def p_group(p_u, p, k):
        if k in (1, 2, 3):
            return p_u[p, 32 * k:32 * k + 32, :]
        pm = p_u[p, 0:32, :]
        new = pm & m2_s[...]
        return new if k == 4 else pm ^ new

    def pv_tile(I, p, t, acc):
        zero = jnp.zeros((32, 128), U32)
        b, j = p // 2 % NBUF, p % 2
        wa, wb = [], []
        for k in (2 * t, 2 * t + 1):
            ek = p_group(pu_bufs[b][0], j, k) if k < 5 else zero
            ok = p_group(pu_bufs[b][1], j, k - 1) if k > 0 else zero
            wa.append(jnp.where(lo32, ek, ok))
            wb.append(jnp.where(lo32, ok, ek))
        out = []
        for s, (w, l_ref) in enumerate(zip((wa, wb), l_bufs[b])):
            h = 2 * p + s
            vt = pltpu.bitcast(vt_u[I - 2 + t, 8 * h:8 * h + 8, :], BF)
            ot = jnp.dot(vt, pltpu.bitcast(jnp.concatenate(w, axis=0), BF), preferred_element_type=F32)
            ot = ot if acc is None else acc[s] + ot
            if t == 2:
                o = ot * l_ref[j][0:1]
                if s == 1:
                    o = pltpu.roll(o, 64, 1)
                ot_s[I, 16 * h:16 * h + 16, :] = o.astype(BF)
            out.append(ot)
        return out

    def wo_pieces(b):
        st = {}
        r0 = _mult(b * QB, QB)
        x1_ref, h2_ref = d_bufs[b % 2 if isinstance(b, int) else b.parity]
        b = b if isinstance(b, int) else b.value
        ot = pltpu.bitcast(ot_u[b], BF)
        for n in range(4):
            on_s[n] = ot[n * 128:(n + 1) * 128, :].T

        def p_wo(n):
            def run():
                att = jnp.dot(_ldp(on_s, 0, 4), _ldp(wo_v, n, n + 1), preferred_element_type=F32)
                st.setdefault("att", []).append(att)
                if n == 3:
                    att = jnp.concatenate(st["att"], axis=1)
                    x1 = x_v[pl.ds(r0, QB), :].astype(F32) + mod_v[0:1, 2 * D:3 * D] * att
                    x1_ref[...] = x1
                    h2 = _layernorm_mod(x1, mod_v[0:1, 3 * D:4 * D], 1.0 + mod_v[0:1, 4 * D:5 * D])
                    for g in range(4):
                        h2_ref[g] = h2[:, g * 128:(g + 1) * 128].astype(BF)
            return run

        return [p_wo(n) for n in range(4)]

    def ffn_pieces(b):
        st = {}
        r0 = _mult(b * QB, QB)
        x1_ref, h2_ref = d_bufs[b % 2 if isinstance(b, int) else b.parity]

        def p_w1(n):
            def run():
                f = jnp.dot(_ldp(h2_ref, 0, 4), _ldp(w1_v, n, n + 1), preferred_element_type=F32)
                st.setdefault("f", []).append(jnp.maximum(f, 0.0).astype(BF))
            return run

        def p_w2(c, n0, n1):
            k0, k1 = 4 * c, min(4 * c + 4, 14)

            def run():
                f = jnp.concatenate(st["f"][k0:k1], axis=1)
                y = jnp.dot(f, _ldp(w2_v, n0, n1, k0 * 128, k1 * 128), preferred_element_type=F32)
                for n in range(n0, n1):
                    yn = y[:, (n - n0) * 128:(n - n0 + 1) * 128]
                    if c > 0:
                        yn = st["y", n] + yn
                    st["y", n] = yn
                    if c == 3:
                        cs = slice(n * 128, (n + 1) * 128)
                        o_v[pl.ds(r0, QB), cs] = (
                            x1_ref[:, cs] + mod_v[0:1, 5 * D + n * 128:5 * D + (n + 1) * 128] * yn
                        ).astype(BF)
            return run

        w1 = [p_w1(n) for n in range(14)]
        w2 = {(c, n): p_w2(c, n, n + 1) for c in range(3) for n in range(4)}
        seq = w1[0:4]
        for i in range(8):
            seq += [w1[4 + i], w2[(i // 4, i % 4)]]
        seq += [w1[12], w1[13], w2[(2, 0)], w2[(2, 1)], w2[(2, 2)], w2[(2, 3)],
                p_w2(3, 0, 2), p_w2(3, 2, 4)]
        return seq

    d_bufs = ((x1a, h2a), (x1b, h2b))

    def out_copy(b):
        r0 = _mult(b * QB, QB)
        return pltpu.make_async_copy(o_v.at[pl.ds(r0, QB), :], o_hbm.at[0, pl.ds(r0, QB), :], osems.at[b])

    def nop():
        pass

    def step(I, pieces):
        last = isinstance(I, int) and I == NQ - 1
        t0 = first_valid(I, 0) // 128
        for g in range(NG):
            if not (last and g + LQ >= NG):
                gq, Iq = (g + LQ) % NG, I + (g + LQ) // NG
                for p in (2 * gq, 2 * gq + 1):
                    for e in range(2):
                        qk(Iq, e, p)
            sms = [nop, nop]
            if not (last and g + LS >= NG):
                gs, Is = (g + LS) % NG, I + (g + LS) // NG
                sms = [lambda p=p, Is=Is: sm(Is, p) for p in (2 * gs, 2 * gs + 1)]
            acc = {p: None for p in (2 * g, 2 * g + 1)}
            for t in range(4):
                if t in (2, 3):
                    sms[t - 2]()
                pieces[4 * g + t]()
                if t0 <= t < 3:
                    for p in acc:
                        acc[p] = pv_tile(I, p, t, acc[p])

    for d in [d_wm1] + d_wo + d_w1 + d_w2:
        d.wait()

    def mod2(n):
        def run():
            cs = slice(2 * D + n * 128, 2 * D + (n + 1) * 128)
            mod_v[:, cs] = jnp.dot(sc16, wmod_v[:, cs], preferred_element_type=F32)[0:8]
        return run

    def blk(I, k, parity):
        return I - k if isinstance(I, int) else _Blk(I - k, (parity - k) % 2)

    def full_step(I, parity=None):
        wo = wo_pieces(blk(I, 1, parity))
        ffn = ffn_pieces(blk(I, 2, parity))
        step(I, ffn[0:WOPOS] + wo + ffn[WOPOS:])
        out_copy(I - 2).start()

    for p in range(2 * LQ):
        for e in range(2):
            qk(0, e, p)
    for p in range(2 * LS):
        sm(0, p)
    step(0, [mod2(n // 2) if n % 2 == 0 else nop for n in range(32)])
    wo0 = wo_pieces(0)
    step(1, [nop] * WOPOS + wo0 + [nop] * (28 - WOPOS))

    def body(i, carry):
        full_step(2 * i, 0)
        full_step(2 * i + 1, 1)
        return carry

    jax.lax.fori_loop(1, NQ // 2 - 1, body, 0)
    full_step(NQ - 2)
    full_step(NQ - 1)
    wo = wo_pieces(NQ - 1)
    ffn = ffn_pieces(NQ - 2)
    for p in wo + ffn:
        p()
    out_copy(NQ - 2).start()
    for p in ffn_pieces(NQ - 1):
        p()
    out_copy(NQ - 1).start()
    for b in range(NQ):
        out_copy(b).wait()


@jax.jit
def pallas_adaLN_cond__sliding_block__dense_activation_relu__prompt_kernel(
    A_x: jax.Array,
    A_wqkv: jax.Array,
    A_wo: jax.Array,
    B_x: jax.Array,
    B_w1: jax.Array,
    B_w2: jax.Array,
    c: jax.Array,
    w_mod: jax.Array,
):
    del B_x
    scratch = [
        pltpu.VMEM((S, D), BF),
        pltpu.VMEM((12, D, 128), BF),
        pltpu.VMEM((4, D, 128), BF),
        pltpu.VMEM((14, D, 128), BF),
        pltpu.VMEM((4, DFF, 128), BF),
        pltpu.VMEM((1, D), BF),
        pltpu.VMEM((D, 6 * D), BF),
        pltpu.VMEM((8, 6 * D), F32),
        pltpu.VMEM((4, TM, 128), BF),
        pltpu.VMEM((4, TM, 128), BF),
        pltpu.VMEM((4, S, 128), BF),
        pltpu.VMEM((NQ, D, 128), BF),
        pltpu.VMEM((NQ, D, 128), BF),
        pltpu.VMEM((NQ, D, 128), BF),
        pltpu.VMEM((32, 128), U32),
        pltpu.VMEM((S, D), BF),
        pltpu.VMEM((4, QB, 128), BF),
        pltpu.VMEM((QB, D), F32),
        pltpu.VMEM((4, QB, 128), BF),
        pltpu.VMEM((QB, D), F32),
        pltpu.VMEM((4, QB, 128), BF),
        pltpu.SemaphoreType.DMA((50,)),
        pltpu.SemaphoreType.DMA((NQ,)),
    ] + NBUF * [
        pltpu.VMEM((2, 256, 128), F32),
        pltpu.VMEM((2, 8, 128), F32),
        pltpu.VMEM((2, 256, 128), F32),
        pltpu.VMEM((2, 8, 128), F32),
        pltpu.VMEM((2, 256, 128), BF),
        pltpu.VMEM((2, 256, 128), BF),
        pltpu.VMEM((2, 8, 128), F32),
        pltpu.VMEM((2, 8, 128), F32),
    ]
    return pl.pallas_call(
        _kernel,
        out_shape=jax.ShapeDtypeStruct((1, S, D), BF),
        in_specs=[pl.BlockSpec(memory_space=pl.ANY)] * 7,
        out_specs=pl.BlockSpec(memory_space=pl.ANY),
        scratch_shapes=scratch,
        compiler_params=pltpu.CompilerParams(vmem_limit_bytes=100 * 1024 * 1024),
        name="adaln_swa_ffn",
    )(A_x, A_wqkv, A_wo, B_w1, B_w2, c, w_mod)
```

```python
import jax
import jax.numpy as jnp
import jax.experimental.pallas as pl
import jax.experimental.pallas.tpu as pltpu

S = 2048
D = 512
H = 32
DH = 16
WIN = 256
DFF = 1792
EPS = 1e-5
NEG = -1e30
QSCALE = (DH ** -0.5) * 1.4426950408889634

TM = 256
NB = S // TM
QB = 128
NQ = S // QB
NP = H // 2
NG = 8
NHB = 8
NBUF = 2
LS = 1
SMT = (2, 3)
WOPOS = 14
LQ = 2

BF = jnp.bfloat16
F32 = jnp.float32
U32 = jnp.uint32

TT = (((0,), (1,)), ((), ()))


def _ldp(ref, p0, p1, r0=None, r1=None):
    u = ref.bitcast(U32)
    if r0 is None:
        r0, r1 = 0, ref.shape[1]
    return pltpu.bitcast(
        jnp.concatenate([u[p, r0 // 2:r1 // 2, :] for p in range(p0, p1)], axis=1), BF)


def _mult(x, m):
    return x if isinstance(x, int) else pl.multiple_of(x, m)


class _Blk:
    def __init__(self, value, parity):
        self.value, self.parity = value, parity

    def __mul__(self, k):
        return self.value * k


def _normalize(x):
    m = jnp.mean(x, axis=-1, keepdims=True)
    xc = x - m
    v = jnp.mean(xc * xc, axis=-1, keepdims=True)
    return xc * jax.lax.rsqrt(v + EPS)


def _layernorm_mod(x, shift, scale1p):
    return _normalize(x) * scale1p + shift


def _kernel(x_hbm, wqkv_hbm, wo_hbm, w1_hbm, w2_hbm, c_hbm, wmod_hbm, o_hbm,
            x_v, wqkv_v, wo_v, w1_v, w2_v, c_v, wmod_v, mod_v,
            ha, hb, k0_s, k1_s, k2_s, k3_s, qt_s, vt_s, ot_s, m2_s,
            o_v, on_s, x1a, h2a, x1b, h2b, sems, *bufs):
    def cp(src, dst, i):
        return pltpu.make_async_copy(src, dst, sems.at[i])

    def panels(src, dst, n0, n1, sem):
        return [cp(src.at[:, pl.ds(n * 128, 128)], dst.at[n], sem) for n in range(n0, n1)]

    def x_rows(r0, r1, sem):
        return cp(x_hbm.at[0, pl.ds(r0, r1 - r0), :], x_v.at[pl.ds(r0, r1 - r0), :], sem)

    d_c = cp(c_hbm, c_v, 0)
    d_x0 = x_rows(0, TM, 0)
    d_wm0 = cp(wmod_hbm.at[:, pl.ds(0, 2 * D)], wmod_v.at[:, pl.ds(0, 2 * D)], 1)
    d_wk = panels(wqkv_hbm, wqkv_v, 4, 8, 2)
    d_x1 = x_rows(TM, 2 * TM, 2)
    d_wq = panels(wqkv_hbm, wqkv_v, 0, 4, 3)
    d_wv = panels(wqkv_hbm, wqkv_v, 8, 12, 3)
    d_x2 = x_rows(2 * TM, 3 * TM, 3)
    d_x3 = x_rows(3 * TM, S, 4)
    d_wm1 = cp(wmod_hbm.at[:, pl.ds(2 * D, 4 * D)], wmod_v.at[:, pl.ds(2 * D, 4 * D)], 0)
    d_wo = panels(wo_hbm, wo_v, 0, 4, 0)
    d_w1 = panels(w1_hbm, w1_v, 0, 14, 0)
    d_w2 = panels(w2_hbm, w2_v, 0, 4, 0)
    for d in [d_c, d_x0, d_wm0] + d_wk + [d_x1] + d_wq + d_wv + [d_x2, d_x3]:
        d.start()

    bufs = [bufs[8 * b:8 * b + 8] for b in range(NBUF + NHB)]
    s_bufs = [((se, me), (so, mo)) for se, me, so, mo, _, _, _, _ in bufs]
    p_bufs = [b[4:6] for b in bufs]
    l_bufs = [b[6:8] for b in bufs]
    for b in p_bufs[:NBUF]:
        for p_ref in b:
            p_ref[...] = jnp.zeros((2, 256, 128), BF)
    i2 = 2 * jax.lax.broadcasted_iota(jnp.int32, (32, 128), 0)
    al = jax.lax.broadcasted_iota(jnp.int32, (32, 128), 1) & 63
    m2_s[...] = (jnp.where(i2 <= al, jnp.uint32(0xFFFF), jnp.uint32(0))
                 | jnp.where(i2 + 1 <= al, jnp.uint32(0xFFFF0000), jnp.uint32(0)))

    d_c.wait()
    d_x0.wait()
    cf = c_v[...].astype(F32)
    sc = (cf * (1.0 / (1.0 + jnp.exp(-cf)))).astype(BF)
    sc16 = jnp.broadcast_to(sc, (16, D))
    n0 = _normalize(x_v[0:TM, :].astype(F32))
    d_wm0.wait()
    mod_v[:, 0:2 * D] = jnp.dot(sc16, wmod_v[:, 0:2 * D], preferred_element_type=F32)[0:8]

    def put_h(n, h_ref):
        h = (n * (1.0 + mod_v[0:1, D:2 * D]) + mod_v[0:1, 0:D]).astype(BF)
        for p in range(4):
            h_ref[p] = h[:, p * 128:(p + 1) * 128]

    def ln1(b, h_ref):
        r0 = pl.multiple_of(b * TM, TM)
        put_h(_normalize(x_v[pl.ds(r0, TM), :].astype(F32)), h_ref)

    def proj_k(b, h_cur):
        h = _ldp(h_cur, 0, 4)
        kk = jnp.dot(h, _ldp(wqkv_v, 4, 8), preferred_element_type=F32)
        r0 = _mult(b * TM, TM)
        lane = jax.lax.broadcasted_iota(jnp.int32, (TM, 128), 1)
        odd, hi = (lane & 32) != 0, lane >= 64
        for g in range(4):
            k = kk[:, g * 128:(g + 1) * 128]
            ka = jnp.where(odd, pltpu.roll(k, 32, 1), k)
            kb = jnp.where(odd, k, pltpu.roll(k, 96, 1))
            for kx, s_lo, s_hi in ((ka, k0_s, k2_s), (kb, k1_s, k3_s)):
                kr = pltpu.roll(kx, 64, 1)
                s_lo[g, pl.ds(r0, TM), :] = jnp.where(hi, kr, kx).astype(BF)
                s_hi[g, pl.ds(r0, TM), :] = jnp.where(hi, kx, kr).astype(BF)

    def proj_qv(b, h_cur):
        h = _ldp(h_cur, 0, 4)
        wqv = jnp.concatenate([_ldp(wqkv_v, 0, 4), _ldp(wqkv_v, 8, 12)], axis=1)
        qv = jax.lax.dot_general(wqv, h, TT, preferred_element_type=F32)
        for t in range(TM // QB):
            q = qv[0:D, t * QB:(t + 1) * QB] * QSCALE
            q = jnp.concatenate(
                [q[16 * h:16 * h + 16] if h % 2 == 0 else pltpu.roll(q[16 * h:16 * h + 16], 64, 1)
                 for h in range(H)], axis=0)
            qt_s[b * (TM // QB) + t] = q.astype(BF)
            vt_s[b * (TM // QB) + t] = qv[D:2 * D, t * QB:(t + 1) * QB].astype(BF)

    def proj(b, h_cur, h_nxt):
        ln1(jnp.minimum(b + 1, NB - 1), h_nxt)
        proj_k(b, h_cur)
        proj_qv(b, h_cur)

    put_h(n0, ha)
    for d in d_wk + [d_x1]:
        d.wait()
    proj_k(0, ha)
    ln1(1, hb)
    proj_k(1, hb)
    for d in d_wq + d_wv + [d_x2]:
        d.wait()
    for d in [d_wm1] + d_wo + d_w1 + d_w2:
        d.start()
    proj_qv(0, ha)
    ln1(2, ha)
    proj_qv(1, hb)
    d_x3.wait()

    def proj_body(b2, carry):
        proj(2 * b2, ha, hb)
        proj(2 * b2 + 1, hb, ha)
        return carry

    jax.lax.fori_loop(1, NB // 2, proj_body, 0)

    lane8 = jax.lax.broadcasted_iota(jnp.int32, (8, 128), 1)
    sub8 = jax.lax.broadcasted_iota(jnp.int32, (8, 128), 0)
    dd = (lane8 & 63) - sub8
    chunk8 = (lane8 >> 4) & 3
    ddc = [jnp.where(chunk8 == c, dd, -128) for c in range(4)]
    slot_gt = [lane8 >= 32 * (c + 1) for c in range(3)]
    grp8 = [(lane8 >> 4) == i for i in range(8)]
    lo8 = lane8 < 64
    lo32 = jax.lax.broadcasted_iota(jnp.int32, (32, 128), 1) < 64
    lo1 = jax.lax.broadcasted_iota(jnp.int32, (1, 128), 1) < 64

    k_us = [r.bitcast(U32) for r in (k0_s, k1_s, k2_s, k3_s)]
    qt_u = qt_s.bitcast(U32)
    vt_u = vt_s.bitcast(U32)
    ot_u = ot_s.bitcast(U32)
    pu_bufs = [[r.bitcast(U32) for r in rs] for rs in p_bufs]

    def buf(I, p):
        return NBUF + p // 2 % NHB if isinstance(I, int) and I < 2 else p // 2 % NBUF

    def first_valid(I, e):
        return max(0, WIN - 64 * (2 * I + e)) if isinstance(I, int) else 0

    def qk(I, e, p):
        s_ref, m_ref = s_bufs[buf(I, p)][e]
        j = p % 2
        g, k_u = p // 4, k_us[p % 4]
        qa = qt_u[I, 16 * p:16 * p + 8, :]
        qb = qt_u[I, 16 * p + 8:16 * p + 16, :]
        zero = jnp.zeros((8, 128), U32)
        ga, gb = (0, 4) if e == 0 else (4, 0)
        parts = []
        for c in range(4):
            parts += [jnp.where(grp8[ga + c], qa, zero), jnp.where(grp8[gb + c], qb, zero)]
        wq = pltpu.bitcast(jnp.concatenate(parts, axis=0), BF)
        lo = first_valid(I, e)
        kb = (2 * I + e) * 32 - WIN // 2

        def krows(o):
            return k_u[g, pl.ds(_mult(kb + o // 2, 8), 8), :]

        mid = [(o, lambda o=o: krows(o)) for o in range(max(lo, 64), WIN, 16)]
        if lo == 0:
            new = [krows(WIN + 16 * r) for r in range(4)]
            old = [krows(16 * r) for r in range(4)]
            diag = jnp.where(slot_gt[1], jnp.where(slot_gt[2], new[3], new[2]),
                             jnp.where(slot_gt[0], new[1], new[0]))
            tri = [("d", lambda: diag)] + [
                (16 * r, lambda r=r: jnp.where(slot_gt[r], new[r], old[r]) if r < 3 else old[r]) for r in range(4)]
            rows = [tri[0]]
            for r in range(4):
                rows += [tri[1 + r]] + mid[3 * r:3 * r + 3]
        else:
            rows = [(16 * r, lambda r=r: krows(WIN + 16 * r)) for r in range(4)] + mid
        kg = pltpu.bitcast(jnp.concatenate([f() for _, f in rows], axis=0), BF)
        st = jnp.dot(kg, wq, preferred_element_type=F32)
        blk = {(o, h): st[16 * i + 8 * h:16 * i + 8 * h + 8] for i, (o, _) in enumerate(rows) for h in range(2)}
        mx = [None, None]
        for o, _ in rows:
            if o == "d":
                continue
            for h in range(2):
                mu = o + 8 * h
                v = blk[o, h]
                if mu < 64:
                    v = jnp.where(ddc[o // 16] >= mu, blk["d", h], v) if lo == 0 else jnp.where(dd >= mu, v, NEG)
                s_ref[j, mu:mu + 8, :] = v
                mx[h] = v if mx[h] is None else jnp.maximum(mx[h], v)
        m = jnp.max(jnp.maximum(mx[0], mx[1]), axis=0, keepdims=True)
        m_ref[j] = jnp.broadcast_to(m, (8, 128))

    def sm(I, p):
        li = []
        b, j = buf(I, p), p % 2
        for e in range(2):
            (s_ref, m_ref), p_ref = s_bufs[b][e], p_bufs[b][e]
            mrow = m_ref[j][0:1]
            lvl = []
            for r in range(16):
                if r < 4 or 16 * r >= first_valid(I, e):
                    pj = jnp.exp2(s_ref[j, 16 * r:16 * r + 16, :] - mrow)
                    p_ref[j, 16 * r:16 * r + 16, :] = pj.astype(BF)
                    lvl.append(pj[0:8] + pj[8:16])
            while len(lvl) > 1:
                lvl = [lvl[i] + lvl[i + 1] if i + 1 < len(lvl) else lvl[i] for i in range(0, len(lvl), 2)]
            tot = lvl[0]
            li.append(1.0 / jnp.sum(tot, axis=0, keepdims=True))
        l_bufs[b][0][j] = jnp.broadcast_to(jnp.where(lo1, li[0], li[1]), (8, 128))
        l_bufs[b][1][j] = jnp.broadcast_to(jnp.where(lo1, li[1], li[0]), (8, 128))

    def p_group(p_u, p, k):
        if k in (1, 2, 3):
            return p_u[p, 32 * k:32 * k + 32, :]
        pm = p_u[p, 0:32, :]
        new = pm & m2_s[...]
        return new if k == 4 else pm ^ new

    def pv_tile(I, p, t, acc):
        zero = jnp.zeros((32, 128), U32)
        b, j = buf(I, p), p % 2
        wa, wb = [], []
        for k in (2 * t, 2 * t + 1):
            ek = p_group(pu_bufs[b][0], j, k) if k < 5 else zero
            ok = p_group(pu_bufs[b][1], j, k - 1) if k > 0 else zero
            wa.append(jnp.where(lo32, ek, ok))
            wb.append(jnp.where(lo32, ok, ek))
        out = []
        for s, (w, l_ref) in enumerate(zip((wa, wb), l_bufs[b])):
            h = 2 * p + s
            vt = pltpu.bitcast(vt_u[I - 2 + t, 8 * h:8 * h + 8, :], BF)
            ot = jnp.dot(vt, pltpu.bitcast(jnp.concatenate(w, axis=0), BF), preferred_element_type=F32)
            ot = ot if acc is None else acc[s] + ot
            if t == 2:
                o = ot * l_ref[j][0:1]
                if s == 1:
                    o = pltpu.roll(o, 64, 1)
                ot_s[I, 16 * h:16 * h + 16, :] = o.astype(BF)
            out.append(ot)
        return out

    def wo_pieces(b):
        st = {}
        r0 = _mult(b * QB, QB)
        x1_ref, h2_ref = d_bufs[b % 2 if isinstance(b, int) else b.parity]
        b = b if isinstance(b, int) else b.value
        ot = pltpu.bitcast(ot_u[b], BF)
        for n in range(4):
            on_s[n] = ot[n * 128:(n + 1) * 128, :].T

        def p_wo(n):
            def run():
                att = jnp.dot(_ldp(on_s, 0, 4), _ldp(wo_v, n, n + 1), preferred_element_type=F32)
                st.setdefault("att", []).append(att)
                if n == 3:
                    att = jnp.concatenate(st["att"], axis=1)
                    x1 = x_v[pl.ds(r0, QB), :].astype(F32) + mod_v[0:1, 2 * D:3 * D] * att
                    x1_ref[...] = x1
                    h2 = _layernorm_mod(x1, mod_v[0:1, 3 * D:4 * D], 1.0 + mod_v[0:1, 4 * D:5 * D])
                    for g in range(4):
                        h2_ref[g] = h2[:, g * 128:(g + 1) * 128].astype(BF)
            return run

        return [p_wo(n) for n in range(4)]

    def ffn_pieces(b):
        st = {}
        r0 = _mult(b * QB, QB)
        x1_ref, h2_ref = d_bufs[b % 2 if isinstance(b, int) else b.parity]

        def p_w1(n):
            def run():
                f = jnp.dot(_ldp(h2_ref, 0, 4), _ldp(w1_v, n, n + 1), preferred_element_type=F32)
                st.setdefault("f", []).append(jnp.maximum(f, 0.0).astype(BF))
            return run

        def p_w2(c, n0, n1):
            k0, k1 = 4 * c, min(4 * c + 4, 14)

            def run():
                f = jnp.concatenate(st["f"][k0:k1], axis=1)
                y = jnp.dot(f, _ldp(w2_v, n0, n1, k0 * 128, k1 * 128), preferred_element_type=F32)
                for n in range(n0, n1):
                    yn = y[:, (n - n0) * 128:(n - n0 + 1) * 128]
                    if c > 0:
                        yn = st["y", n] + yn
                    st["y", n] = yn
                    if c == 3:
                        cs = slice(n * 128, (n + 1) * 128)
                        o_v[pl.ds(r0, QB), cs] = (
                            x1_ref[:, cs] + mod_v[0:1, 5 * D + n * 128:5 * D + (n + 1) * 128] * yn
                        ).astype(BF)
            return run

        w1 = [p_w1(n) for n in range(14)]
        w2 = {(c, n): p_w2(c, n, n + 1) for c in range(3) for n in range(4)}
        seq = w1[0:4]
        for i in range(8):
            seq += [w1[4 + i], w2[(i // 4, i % 4)]]
        seq += [w1[12], w1[13], w2[(2, 0)], w2[(2, 1)], w2[(2, 2)], w2[(2, 3)],
                p_w2(3, 0, 2), p_w2(3, 2, 4)]
        return seq

    d_bufs = ((x1a, h2a), (x1b, h2b))

    def out_copy(b):
        r0 = _mult(b * QB, QB)
        return pltpu.make_async_copy(o_v.at[pl.ds(r0, QB), :], o_hbm.at[0, pl.ds(r0, QB), :], sems.at[1])

    def nop():
        pass

    def step(I, pieces):
        last = isinstance(I, int) and I == NQ - 1
        t0 = first_valid(I, 0) // 128
        for g in range(NG):
            if not (last and g + LQ >= NG):
                gq, Iq = (g + LQ) % NG, I + (g + LQ) // NG
                for p in (2 * gq, 2 * gq + 1):
                    for e in range(2):
                        qk(Iq, e, p)
            sms = [nop, nop]
            if not (last and g + LS >= NG):
                gs, Is = (g + LS) % NG, I + (g + LS) // NG
                sms = [lambda p=p, Is=Is: sm(Is, p) for p in (2 * gs, 2 * gs + 1)]
            acc = {p: None for p in (2 * g, 2 * g + 1)}
            for t in range(4):
                for i, ts in enumerate(SMT):
                    if ts == t:
                        sms[i]()
                pieces[4 * g + t]()
                if t0 <= t < 3:
                    for p in acc:
                        acc[p] = pv_tile(I, p, t, acc[p])

    for d in [d_wm1] + d_wo + d_w1 + d_w2:
        d.wait()

    def mod2(n):
        def run():
            cs = slice(2 * D + n * 128, 2 * D + (n + 1) * 128)
            mod_v[:, cs] = jnp.dot(sc16, wmod_v[:, cs], preferred_element_type=F32)[0:8]
        return run

    def blk(I, k, parity):
        return I - k if isinstance(I, int) else _Blk(I - k, (parity - k) % 2)

    def full_step(I, parity=None):
        wo = wo_pieces(blk(I, 1, parity))
        ffn = ffn_pieces(blk(I, 2, parity))
        step(I, ffn[0:WOPOS] + wo + ffn[WOPOS:])
        out_copy(I - 2).start()

    for p in range(2 * LQ):
        for e in range(2):
            qk(0, e, p)
    for p in range(2 * LS):
        sm(0, p)
    step(0, [mod2(n // 2) if n % 2 == 0 else nop for n in range(32)])
    wo0 = wo_pieces(0)
    step(1, [nop] * WOPOS + wo0 + [nop] * (28 - WOPOS))

    def body(i, carry):
        full_step(2 * i, 0)
        full_step(2 * i + 1, 1)
        return carry

    jax.lax.fori_loop(1, NQ // 2 - 1, body, 0)
    full_step(NQ - 2)
    full_step(NQ - 1)
    wo = wo_pieces(NQ - 1)
    ffn = ffn_pieces(NQ - 2)
    for p in wo + ffn:
        p()
    out_copy(NQ - 2).start()
    for p in ffn_pieces(NQ - 1):
        p()
    out_copy(NQ - 1).start()
    for b in range(NQ):
        out_copy(b).wait()


@jax.jit
def pallas_adaLN_cond__sliding_block__dense_activation_relu__prompt_kernel(
    A_x: jax.Array,
    A_wqkv: jax.Array,
    A_wo: jax.Array,
    B_x: jax.Array,
    B_w1: jax.Array,
    B_w2: jax.Array,
    c: jax.Array,
    w_mod: jax.Array,
):
    del B_x
    scratch = [
        pltpu.VMEM((S, D), BF),
        pltpu.VMEM((12, D, 128), BF),
        pltpu.VMEM((4, D, 128), BF),
        pltpu.VMEM((14, D, 128), BF),
        pltpu.VMEM((4, DFF, 128), BF),
        pltpu.VMEM((1, D), BF),
        pltpu.VMEM((D, 6 * D), BF),
        pltpu.VMEM((8, 6 * D), F32),
        pltpu.VMEM((4, TM, 128), BF),
        pltpu.VMEM((4, TM, 128), BF),
        pltpu.VMEM((4, S, 128), BF),
        pltpu.VMEM((4, S, 128), BF),
        pltpu.VMEM((4, S, 128), BF),
        pltpu.VMEM((4, S, 128), BF),
        pltpu.VMEM((NQ, D, 128), BF),
        pltpu.VMEM((NQ, D, 128), BF),
        pltpu.VMEM((NQ, D, 128), BF),
        pltpu.VMEM((32, 128), U32),
        pltpu.VMEM((S, D), BF),
        pltpu.VMEM((4, QB, 128), BF),
        pltpu.VMEM((QB, D), F32),
        pltpu.VMEM((4, QB, 128), BF),
        pltpu.VMEM((QB, D), F32),
        pltpu.VMEM((4, QB, 128), BF),
        pltpu.SemaphoreType.DMA((5,)),
    ] + (NBUF + NHB) * [
        pltpu.VMEM((2, 256, 128), F32),
        pltpu.VMEM((2, 8, 128), F32),
        pltpu.VMEM((2, 256, 128), F32),
        pltpu.VMEM((2, 8, 128), F32),
        pltpu.VMEM((2, 256, 128), BF),
        pltpu.VMEM((2, 256, 128), BF),
        pltpu.VMEM((2, 8, 128), F32),
        pltpu.VMEM((2, 8, 128), F32),
    ]
    return pl.pallas_call(
        _kernel,
        out_shape=jax.ShapeDtypeStruct((1, S, D), BF),
        in_specs=[pl.BlockSpec(memory_space=pl.ANY)] * 7,
        out_specs=pl.BlockSpec(memory_space=pl.ANY),
        scratch_shapes=scratch,
        compiler_params=pltpu.CompilerParams(vmem_limit_bytes=100 * 1024 * 1024),
        name="adaln_swa_ffn",
    )(A_x, A_wqkv, A_wo, B_w1, B_w2, c, w_mod)
```

```python
import jax
import jax.numpy as jnp
import jax.experimental.pallas as pl
import jax.experimental.pallas.tpu as pltpu

S = 2048
D = 512
H = 32
DH = 16
WIN = 256
DFF = 1792
EPS = 1e-5
NEG = -1e30
QSCALE = (DH ** -0.5) * 1.4426950408889634

TM = 256
NB = S // TM
QB = 128
NQ = S // QB
NP = H // 2
NG = 8
NHB = 8
NBUF = 2
LS = 1
SMT = (0, 1)
WOPOS = 10
WOPOS1 = 6
WOPOST = 4
LQ = 2

BF = jnp.bfloat16
F32 = jnp.float32
U32 = jnp.uint32

TT = (((0,), (1,)), ((), ()))


def _ldp(ref, p0, p1, r0=None, r1=None):
    u = ref.bitcast(U32)
    if r0 is None:
        r0, r1 = 0, ref.shape[1]
    return pltpu.bitcast(
        jnp.concatenate([u[p, r0 // 2:r1 // 2, :] for p in range(p0, p1)], axis=1), BF)


def _mult(x, m):
    return x if isinstance(x, int) else pl.multiple_of(x, m)


class _Blk:
    def __init__(self, value, parity):
        self.value, self.parity = value, parity

    def __mul__(self, k):
        return self.value * k


def _normalize(x):
    m = jnp.mean(x, axis=-1, keepdims=True)
    xc = x - m
    v = jnp.mean(xc * xc, axis=-1, keepdims=True)
    return xc * jax.lax.rsqrt(v + EPS)


def _layernorm_mod(x, shift, scale1p):
    return _normalize(x) * scale1p + shift


def _kernel(x_hbm, wqkv_hbm, wo_hbm, w1_hbm, w2_hbm, c_hbm, wmod_hbm, o_hbm,
            x_v, wqkv_v, wo_v, w1_v, w2_v, c_v, wmod_v, mod_v,
            ha, hb, k0_s, k1_s, k2_s, k3_s, qt_s, vt_s, ot_s, m2_s,
            o_v, on_s, x1a, h2a, fa, x1b, h2b, fb, sems, *bufs):
    def cp(src, dst, i):
        return pltpu.make_async_copy(src, dst, sems.at[i])

    def panels(src, dst, n0, n1, sem):
        return [cp(src.at[:, pl.ds(n * 128, 128)], dst.at[n], sem) for n in range(n0, n1)]

    def x_rows(r0, r1, sem):
        return cp(x_hbm.at[0, pl.ds(r0, r1 - r0), :], x_v.at[pl.ds(r0, r1 - r0), :], sem)

    d_c = cp(c_hbm, c_v, 0)
    d_x0 = x_rows(0, TM, 0)
    d_wm0 = cp(wmod_hbm.at[:, pl.ds(0, 2 * D)], wmod_v.at[:, pl.ds(0, 2 * D)], 1)
    d_wk = panels(wqkv_hbm, wqkv_v, 4, 8, 2)
    d_x1 = x_rows(TM, 2 * TM, 0)
    d_wq = panels(wqkv_hbm, wqkv_v, 0, 4, 3)
    d_wv = panels(wqkv_hbm, wqkv_v, 8, 12, 3)
    d_x2 = x_rows(2 * TM, 3 * TM, 3)
    d_x3 = x_rows(3 * TM, S, 4)
    d_wm1 = cp(wmod_hbm.at[:, pl.ds(2 * D, 4 * D)], wmod_v.at[:, pl.ds(2 * D, 4 * D)], 0)
    d_wo = panels(wo_hbm, wo_v, 0, 4, 0)
    d_w1 = panels(w1_hbm, w1_v, 0, 14, 0)
    d_w2 = panels(w2_hbm, w2_v, 0, 4, 0)
    for d in [d_c, d_x0, d_x1, d_wm0] + d_wk + d_wq + d_wv + [d_x2, d_x3]:
        d.start()

    bufs = [bufs[8 * b:8 * b + 8] for b in range(NBUF + NHB)]
    s_bufs = [((se, me), (so, mo)) for se, me, so, mo, _, _, _, _ in bufs]
    p_bufs = [b[4:6] for b in bufs]
    l_bufs = [b[6:8] for b in bufs]
    for b in p_bufs[:NBUF]:
        for p_ref in b:
            p_ref[...] = jnp.zeros((2, 256, 128), BF)
    i2 = 2 * jax.lax.broadcasted_iota(jnp.int32, (32, 128), 0)
    al = jax.lax.broadcasted_iota(jnp.int32, (32, 128), 1) & 63
    m2_s[...] = (jnp.where(i2 <= al, jnp.uint32(0xFFFF), jnp.uint32(0))
                 | jnp.where(i2 + 1 <= al, jnp.uint32(0xFFFF0000), jnp.uint32(0)))

    d_c.wait()
    d_x0.wait()
    d_x1.wait()
    cf = c_v[...].astype(F32)
    sc = (cf * (1.0 / (1.0 + jnp.exp(-cf)))).astype(BF)
    sc16 = jnp.broadcast_to(sc, (16, D))
    n0 = _normalize(x_v[0:TM, :].astype(F32))
    n1 = _normalize(x_v[TM:2 * TM, :].astype(F32))
    d_wm0.wait()
    mod_v[:, 0:2 * D] = jnp.dot(sc16, wmod_v[:, 0:2 * D], preferred_element_type=F32)[0:8]

    def put_h(n, h_ref):
        h = (n * (1.0 + mod_v[0:1, D:2 * D]) + mod_v[0:1, 0:D]).astype(BF)
        for p in range(4):
            h_ref[p] = h[:, p * 128:(p + 1) * 128]

    def ln1(b, h_ref):
        r0 = pl.multiple_of(b * TM, TM)
        put_h(_normalize(x_v[pl.ds(r0, TM), :].astype(F32)), h_ref)

    def proj_k(b, h_cur):
        h = _ldp(h_cur, 0, 4)
        kk = jnp.dot(h, _ldp(wqkv_v, 4, 8), preferred_element_type=F32)
        r0 = _mult(b * TM, TM)
        lane = jax.lax.broadcasted_iota(jnp.int32, (TM, 128), 1)
        odd, hi = (lane & 32) != 0, lane >= 64
        for g in range(4):
            k = kk[:, g * 128:(g + 1) * 128]
            ka = jnp.where(odd, pltpu.roll(k, 32, 1), k)
            kb = jnp.where(odd, k, pltpu.roll(k, 96, 1))
            for kx, s_lo, s_hi in ((ka, k0_s, k2_s), (kb, k1_s, k3_s)):
                kr = pltpu.roll(kx, 64, 1)
                s_lo[g, pl.ds(r0, TM), :] = jnp.where(hi, kr, kx).astype(BF)
                s_hi[g, pl.ds(r0, TM), :] = jnp.where(hi, kx, kr).astype(BF)

    def proj_qv(b, h_cur):
        h = _ldp(h_cur, 0, 4)
        wqv = jnp.concatenate([_ldp(wqkv_v, 0, 4), _ldp(wqkv_v, 8, 12)], axis=1)
        qv = jax.lax.dot_general(wqv, h, TT, preferred_element_type=F32)
        for t in range(TM // QB):
            q = qv[0:D, t * QB:(t + 1) * QB] * QSCALE
            q = jnp.concatenate(
                [q[16 * h:16 * h + 16] if h % 2 == 0 else pltpu.roll(q[16 * h:16 * h + 16], 64, 1)
                 for h in range(H)], axis=0)
            qt_s[b * (TM // QB) + t] = q.astype(BF)
            vt_s[b * (TM // QB) + t] = qv[D:2 * D, t * QB:(t + 1) * QB].astype(BF)

    def proj(b, h_cur, h_nxt):
        ln1(jnp.minimum(b + 1, NB - 1), h_nxt)
        proj_k(b, h_cur)
        proj_qv(b, h_cur)

    put_h(n0, ha)
    put_h(n1, hb)
    for d in d_wk:
        d.wait()
    for d in [d_wm1] + d_wo + d_w1 + d_w2:
        d.start()
    proj_k(0, ha)
    proj_k(1, hb)
    for d in d_wq + d_wv + [d_x2]:
        d.wait()
    proj_qv(0, ha)
    ln1(2, ha)
    proj_qv(1, hb)
    d_x3.wait()

    def proj_body(b2, carry):
        proj(2 * b2, ha, hb)
        proj(2 * b2 + 1, hb, ha)
        return carry

    jax.lax.fori_loop(1, NB // 2, proj_body, 0)

    lane8 = jax.lax.broadcasted_iota(jnp.int32, (8, 128), 1)
    sub8 = jax.lax.broadcasted_iota(jnp.int32, (8, 128), 0)
    dd = (lane8 & 63) - sub8
    chunk8 = (lane8 >> 4) & 3
    ddc = [jnp.where(chunk8 == c, dd, -128) for c in range(4)]
    slot_gt = [lane8 >= 32 * (c + 1) for c in range(3)]
    grp8 = [(lane8 >> 4) == i for i in range(8)]
    lo32 = jax.lax.broadcasted_iota(jnp.int32, (32, 128), 1) < 64
    lo1 = jax.lax.broadcasted_iota(jnp.int32, (1, 128), 1) < 64

    k_us = [r.bitcast(U32) for r in (k0_s, k1_s, k2_s, k3_s)]
    qt_u = qt_s.bitcast(U32)
    vt_u = vt_s.bitcast(U32)
    ot_u = ot_s.bitcast(U32)
    pu_bufs = [[r.bitcast(U32) for r in rs] for rs in p_bufs]

    def buf(I, p):
        return NBUF + p // 2 % NHB if isinstance(I, int) and I < 2 else p // 2 % NBUF

    def first_valid(I, e):
        return max(0, WIN - 64 * (2 * I + e)) if isinstance(I, int) else 0

    def qk(I, e, p):
        s_ref, m_ref = s_bufs[buf(I, p)][e]
        j = p % 2
        g, k_u = p // 4, k_us[p % 4]
        qa = qt_u[I, 16 * p:16 * p + 8, :]
        qb = qt_u[I, 16 * p + 8:16 * p + 16, :]
        zero = jnp.zeros((8, 128), U32)
        ga, gb = (0, 4) if e == 0 else (4, 0)
        parts = []
        for c in range(4):
            parts += [jnp.where(grp8[ga + c], qa, zero), jnp.where(grp8[gb + c], qb, zero)]
        wq = pltpu.bitcast(jnp.concatenate(parts, axis=0), BF)
        lo = first_valid(I, e)
        kb = (2 * I + e) * 32 - WIN // 2

        def krows(o):
            return k_u[g, pl.ds(_mult(kb + o // 2, 8), 8), :]

        mid = [(o, lambda o=o: krows(o)) for o in range(max(lo, 64), WIN, 16)]
        if lo == 0:
            new = [krows(WIN + 16 * r) for r in range(4)]
            old = [krows(16 * r) for r in range(4)]
            diag = jnp.where(slot_gt[1], jnp.where(slot_gt[2], new[3], new[2]),
                             jnp.where(slot_gt[0], new[1], new[0]))
            tri = [("d", lambda: diag)] + [
                (16 * r, lambda r=r: jnp.where(slot_gt[r], new[r], old[r]) if r < 3 else old[r]) for r in range(4)]
            rows = mid + tri
        else:
            rows = [(16 * r, lambda r=r: krows(WIN + 16 * r)) for r in range(4)] + mid
        kg = pltpu.bitcast(jnp.concatenate([f() for _, f in rows], axis=0), BF)
        st = jnp.dot(kg, wq, preferred_element_type=F32)
        blk = {(o, h): st[16 * i + 8 * h:16 * i + 8 * h + 8] for i, (o, _) in enumerate(rows) for h in range(2)}
        mx = [None, None]
        for o, _ in rows:
            if o == "d":
                continue
            for h in range(2):
                mu = o + 8 * h
                v = blk[o, h]
                if mu < 64:
                    v = jnp.where(ddc[o // 16] >= mu, blk["d", h], v) if lo == 0 else jnp.where(dd >= mu, v, NEG)
                s_ref[j, mu:mu + 8, :] = v
                mx[h] = v if mx[h] is None else jnp.maximum(mx[h], v)
        m = jnp.max(jnp.maximum(mx[0], mx[1]), axis=0, keepdims=True)
        m_ref[j] = jnp.broadcast_to(m, (8, 128))

    def sm(I, p):
        li = []
        b, j = buf(I, p), p % 2
        for e in range(2):
            (s_ref, m_ref), p_ref = s_bufs[b][e], p_bufs[b][e]
            mrow = m_ref[j][0:1]
            lvl = []
            for r in range(16):
                if r < 4 or 16 * r >= first_valid(I, e):
                    pj = jnp.exp2(s_ref[j, 16 * r:16 * r + 16, :] - mrow)
                    p_ref[j, 16 * r:16 * r + 16, :] = pj.astype(BF)
                    lvl.append(pj[0:8] + pj[8:16])
            while len(lvl) > 1:
                lvl = [lvl[i] + lvl[i + 1] if i + 1 < len(lvl) else lvl[i] for i in range(0, len(lvl), 2)]
            tot = lvl[0]
            li.append(1.0 / jnp.sum(tot, axis=0, keepdims=True))
        l_bufs[b][0][j] = jnp.broadcast_to(jnp.where(lo1, li[0], li[1]), (8, 128))
        l_bufs[b][1][j] = jnp.broadcast_to(jnp.where(lo1, li[1], li[0]), (8, 128))

    def p_group(p_u, p, k):
        if k in (1, 2, 3):
            return p_u[p, 32 * k:32 * k + 32, :]
        pm = p_u[p, 0:32, :]
        new = pm & m2_s[...]
        return new if k == 4 else pm ^ new

    def pv_tile(I, p, t, acc):
        zero = jnp.zeros((32, 128), U32)
        b, j = buf(I, p), p % 2
        wa, wb = [], []
        for k in (2 * t, 2 * t + 1):
            ek = p_group(pu_bufs[b][0], j, k) if k < 5 else zero
            ok = p_group(pu_bufs[b][1], j, k - 1) if k > 0 else zero
            wa.append(jnp.where(lo32, ek, ok))
            wb.append(jnp.where(lo32, ok, ek))
        out = []
        for s, (w, l_ref) in enumerate(zip((wa, wb), l_bufs[b])):
            h = 2 * p + s
            vt = pltpu.bitcast(vt_u[I - 2 + t, 8 * h:8 * h + 8, :], BF)
            ot = jnp.dot(vt, pltpu.bitcast(jnp.concatenate(w, axis=0), BF), preferred_element_type=F32)
            ot = ot if acc is None else acc[s] + ot
            if t == 2:
                o = ot * l_ref[j][0:1]
                if s == 1:
                    o = pltpu.roll(o, 64, 1)
                ot_s[I, 16 * h:16 * h + 16, :] = o.astype(BF)
            out.append(ot)
        return out

    def wo_pieces(b):
        st = {}
        r0 = _mult(b * QB, QB)
        x1_ref, h2_ref, _ = d_bufs[b % 2 if isinstance(b, int) else b.parity]
        b = b if isinstance(b, int) else b.value
        ot = pltpu.bitcast(ot_u[b], BF)
        for n in range(4):
            on_s[n] = ot[n * 128:(n + 1) * 128, :].T

        def p_wo(n):
            def run():
                att = jnp.dot(_ldp(on_s, 0, 4), _ldp(wo_v, n, n + 1), preferred_element_type=F32)
                st.setdefault("att", []).append(att)
                if n == 3:
                    att = jnp.concatenate(st["att"], axis=1)
                    x1 = x_v[pl.ds(r0, QB), :].astype(F32) + mod_v[0:1, 2 * D:3 * D] * att
                    x1_ref[...] = x1
                    h2 = _layernorm_mod(x1, mod_v[0:1, 3 * D:4 * D], 1.0 + mod_v[0:1, 4 * D:5 * D])
                    for g in range(4):
                        h2_ref[g] = h2[:, g * 128:(g + 1) * 128].astype(BF)
            return run

        return [p_wo(n) for n in range(4)]

    def w1_pieces(b):
        _, h2_ref, f_ref = d_bufs[b % 2 if isinstance(b, int) else b.parity]

        def p_w1(n):
            def run():
                f = jnp.dot(_ldp(h2_ref, 0, 4), _ldp(w1_v, n, n + 1), preferred_element_type=F32)
                f_ref[n] = jnp.maximum(f, 0.0).astype(BF)
            return run

        return [p_w1(n) for n in range(14)]

    def w2_pieces(b):
        st = {}
        r0 = _mult(b * QB, QB)
        x1_ref, _, f_ref = d_bufs[b % 2 if isinstance(b, int) else b.parity]

        def p_w2(c, n0, n1):
            k0, k1 = 4 * c, min(4 * c + 4, 14)

            def run():
                y = jnp.dot(_ldp(f_ref, k0, k1), _ldp(w2_v, n0, n1, k0 * 128, k1 * 128),
                            preferred_element_type=F32)
                for n in range(n0, n1):
                    yn = y[:, (n - n0) * 128:(n - n0 + 1) * 128]
                    if c > 0:
                        yn = st["y", n] + yn
                    st["y", n] = yn
                    if c == 3:
                        cs = slice(n * 128, (n + 1) * 128)
                        o_v[pl.ds(r0, QB), cs] = (
                            x1_ref[:, cs] + mod_v[0:1, 5 * D + n * 128:5 * D + (n + 1) * 128] * yn
                        ).astype(BF)
            return run

        seq = []
        for n0 in (0, 2):
            seq += [p_w2(c, n, n + 1) for n in (n0, n0 + 1) for c in range(3)] + [p_w2(3, n0, n0 + 2)]
        return seq

    d_bufs = ((x1a, h2a, fa), (x1b, h2b, fb))

    def out_copy(b):
        r0 = _mult(b * QB, QB)
        return pltpu.make_async_copy(o_v.at[pl.ds(r0, QB), :], o_hbm.at[0, pl.ds(r0, QB), :], sems.at[1])

    def nop():
        pass

    def step(I, pieces):
        last = isinstance(I, int) and I == NQ - 1
        t0 = first_valid(I, 0) // 128
        for g in range(NG):
            if not (last and g + LQ >= NG):
                gq, Iq = (g + LQ) % NG, I + (g + LQ) // NG
                for p in (2 * gq, 2 * gq + 1):
                    for e in range(2):
                        qk(Iq, e, p)
            sms = [nop, nop]
            if not (last and g + LS >= NG):
                gs, Is = (g + LS) % NG, I + (g + LS) // NG
                sms = [lambda p=p, Is=Is: sm(Is, p) for p in (2 * gs, 2 * gs + 1)]
            acc = {p: None for p in (2 * g, 2 * g + 1)}
            for t in range(4):
                for i, ts in enumerate(SMT):
                    if ts == t:
                        sms[i]()
                pieces[4 * g + t]()
                if t0 <= t < 3:
                    for p in acc:
                        acc[p] = pv_tile(I, p, t, acc[p])

    for d in [d_wm1] + d_wo + d_w1 + d_w2:
        d.wait()

    def mod2(n):
        def run():
            cs = slice(2 * D + n * 128, 2 * D + (n + 1) * 128)
            mod_v[:, cs] = jnp.dot(sc16, wmod_v[:, cs], preferred_element_type=F32)[0:8]
        return run

    def blk(I, k, parity):
        return I - k if isinstance(I, int) else _Blk(I - k, (parity - k) % 2)

    def full_step(I, parity=None):
        wo = wo_pieces(blk(I, 1, parity))
        w2 = w2_pieces(blk(I, 2, parity))
        step(I, w2[0:WOPOS] + wo + w2[WOPOS:] + w1_pieces(blk(I, 1, parity)))
        out_copy(I - 2).start()

    for p in range(2 * LQ):
        for e in range(2):
            qk(0, e, p)
    for p in range(2 * LS):
        sm(0, p)
    step(0, [mod2(n // 2) if n % 2 == 0 else nop for n in range(32)])
    wo0 = wo_pieces(0)
    step(1, [nop] * WOPOS1 + wo0 + [nop] * (14 - WOPOS1) + w1_pieces(0))

    def body(i, carry):
        full_step(2 * i, 0)
        full_step(2 * i + 1, 1)
        return carry

    jax.lax.fori_loop(1, NQ // 2 - 1, body, 0)
    full_step(NQ - 2)
    full_step(NQ - 1)
    wo = wo_pieces(NQ - 1)
    w2 = w2_pieces(NQ - 2)
    for p in w2[:WOPOST] + wo + w2[WOPOST:]:
        p()
    out_copy(NQ - 2).start()
    r0 = (NQ - 1) * QB
    last = [pltpu.make_async_copy(o_v.at[pl.ds(r0, QB), pl.ds(c0, D // 2)],
                                  o_hbm.at[0, pl.ds(r0, QB), pl.ds(c0, D // 2)], sems.at[1])
            for c0 in (0, D // 2)]
    w2 = w2_pieces(NQ - 1)
    for p in w1_pieces(NQ - 1) + w2[:7]:
        p()
    last[0].start()
    for p in w2[7:]:
        p()
    last[1].start()
    for b in range(NQ - 1):
        out_copy(b).wait()
    for d in last:
        d.wait()


@jax.jit
def pallas_adaLN_cond__sliding_block__dense_activation_relu__prompt_kernel(
    A_x: jax.Array,
    A_wqkv: jax.Array,
    A_wo: jax.Array,
    B_x: jax.Array,
    B_w1: jax.Array,
    B_w2: jax.Array,
    c: jax.Array,
    w_mod: jax.Array,
):
    del B_x
    scratch = [
        pltpu.VMEM((S, D), BF),
        pltpu.VMEM((12, D, 128), BF),
        pltpu.VMEM((4, D, 128), BF),
        pltpu.VMEM((14, D, 128), BF),
        pltpu.VMEM((4, DFF, 128), BF),
        pltpu.VMEM((1, D), BF),
        pltpu.VMEM((D, 6 * D), BF),
        pltpu.VMEM((8, 6 * D), F32),
        pltpu.VMEM((4, TM, 128), BF),
        pltpu.VMEM((4, TM, 128), BF),
        pltpu.VMEM((4, S, 128), BF),
        pltpu.VMEM((4, S, 128), BF),
        pltpu.VMEM((4, S, 128), BF),
        pltpu.VMEM((4, S, 128), BF),
        pltpu.VMEM((NQ, D, 128), BF),
        pltpu.VMEM((NQ, D, 128), BF),
        pltpu.VMEM((NQ, D, 128), BF),
        pltpu.VMEM((32, 128), U32),
        pltpu.VMEM((S, D), BF),
        pltpu.VMEM((4, QB, 128), BF),
        pltpu.VMEM((QB, D), F32),
        pltpu.VMEM((4, QB, 128), BF),
        pltpu.VMEM((14, QB, 128), BF),
        pltpu.VMEM((QB, D), F32),
        pltpu.VMEM((4, QB, 128), BF),
        pltpu.VMEM((14, QB, 128), BF),
        pltpu.SemaphoreType.DMA((5,)),
    ] + (NBUF + NHB) * [
        pltpu.VMEM((2, 256, 128), F32),
        pltpu.VMEM((2, 8, 128), F32),
        pltpu.VMEM((2, 256, 128), F32),
        pltpu.VMEM((2, 8, 128), F32),
        pltpu.VMEM((2, 256, 128), BF),
        pltpu.VMEM((2, 256, 128), BF),
        pltpu.VMEM((2, 8, 128), F32),
        pltpu.VMEM((2, 8, 128), F32),
    ]
    return pl.pallas_call(
        _kernel,
        out_shape=jax.ShapeDtypeStruct((1, S, D), BF),
        in_specs=[pl.BlockSpec(memory_space=pl.ANY)] * 7,
        out_specs=pl.BlockSpec(memory_space=pl.ANY),
        scratch_shapes=scratch,
        compiler_params=pltpu.CompilerParams(vmem_limit_bytes=100 * 1024 * 1024),
        name="adaln_swa_ffn",
    )(A_x, A_wqkv, A_wo, B_w1, B_w2, c, w_mod)
```
